```python
import jax
import jax.numpy as jnp

def _softmax(x, axis=-1):
    return jax.nn.softmax(x, axis=axis)
def _gelu(x):
    return jax.nn.gelu(x, approximate=True)
def _silu(x):
    return jax.nn.silu(x)
def _sigmoid(x):
    return jax.nn.sigmoid(x)
def _layernorm(x, axis=-1, eps=1e-5):
    m = jnp.mean(x, axis=axis, keepdims=True)
    v = jnp.var(x, axis=axis, keepdims=True)
    return (x - m) / jnp.sqrt(v + eps)
def _scatter_add(tgt, idx, src, axis=0):
    return tgt.at[idx].add(src)
def _segment_sum(src, seg, n):
    return jax.ops.segment_sum(src, seg, n)
class _Rng:
    def __init__(self, key):
        self._k = key
    def _next(self):
        self._k, sub = jax.random.split(self._k)
        return sub
    def normal(self, shape):
        return jax.random.normal(self._next(), shape, dtype=jnp.bfloat16)
    def randint(self, lo, hi, shape):
        return jax.random.randint(self._next(), shape, lo, hi, dtype=jnp.int32)
    def uniform(self, shape, lo=0.0, hi=1.0):
        return jax.random.uniform(self._next(), shape, jnp.bfloat16, lo, hi)
    def permutation(self, n):
        return jax.random.permutation(self._next(), n)


kernel_name = 'sequential_preLN__sliding_local_dilated__glu_gated_geglu__prompt'

def setup_inputs():
    _rng = _Rng(jax.random.key(int.from_bytes(__import__("os").urandom(4), "little")))
    _w = (lambda a: (lambda t: t.astype(jnp.bfloat16) if jnp.issubdtype(t.dtype, jnp.floating) else t)(jnp.asarray(a)))
    def _A_setup():
        B, S, D = 1, 2048, 1024
        return {
            "x": _w((lambda *s: _rng.normal(s) * 0.05)(B, S, D)),
            "wqkv": _w((lambda *s: _rng.normal(s) * 0.05)(D, 3 * D)),
            "wo": _w((lambda *s: _rng.normal(s) * 0.05)(D, D)),
        }
    _A_in = _A_setup()

    def _B_setup():
        B, S, Dm, Df = 1, 2048, 1024, 3584
        return {
            "x": _w((lambda *s: _rng.normal(s) * 0.05)(B, S, Dm)),
            "w_gate": _w((lambda *s: _rng.normal(s) * 0.05)(Dm, Df) * (Dm ** -0.5)),
            "w_up": _w((lambda *s: _rng.normal(s) * 0.05)(Dm, Df) * (Dm ** -0.5)),
            "w_down": _w((lambda *s: _rng.normal(s) * 0.05)(Df, Dm) * (Df ** -0.5)),
        }
    _B_in = _B_setup()

    return {
        "A_x": _A_in["x"],
        "A_wqkv": _A_in["wqkv"],
        "A_wo": _A_in["wo"],
        "B_x": _B_in["x"],
        "B_w_gate": _B_in["w_gate"],
        "B_w_up": _B_in["w_up"],
        "B_w_down": _B_in["w_down"],
    }

def reference(A_x, A_wqkv, A_wo, B_x, B_w_gate, B_w_up, B_w_down):
    def _A_ref(x, wqkv, wo):
        B, S, D = x.shape
        H = 32; Dh = D // H
        W, dil = 8, 2
        qkv = (lambda x, *d: x.transpose(*d))((x @ wqkv).reshape(B, S, 3, H, Dh), 2, 0, 3, 1, 4)
        q, k, v = qkv[0], qkv[1], qkv[2]
        scale = Dh ** -0.5
        pos = jnp.arange(S)
        off = jnp.arange(W) * dil
        idx = pos[:, None] - off[None, :]
        mask = idx >= 0
        idx_c = jnp.where(mask, idx, 0).reshape(-1)
        kg = k[:, :, idx_c, :].reshape(B, H, S, W, Dh)
        vg = v[:, :, idx_c, :].reshape(B, H, S, W, Dh)
        logits = jnp.einsum("bhsd,bhswd->bhsw", q, kg) * scale
        logits = jnp.where(mask[None, None, :, :], logits, -1e9)
        attn = _softmax(logits, axis=-1)
        o = jnp.einsum("bhsw,bhswd->bhsd", attn, vg)
        return (lambda x, *d: x.transpose(*d))(o, 0, 2, 1, 3).reshape(B, S, D) @ wo

    def _B_ref(x, w_gate, w_up, w_down):
        g = jnp.einsum("bsd,df->bsf", x, w_gate)
        u = jnp.einsum("bsd,df->bsf", x, w_up)
        h = _gelu(g) * u
        return jnp.einsum("bsf,fd->bsd", h, w_down)

    x = A_x
    h = x + _A_ref(_layernorm(x, axis=-1), A_wqkv, A_wo)
    h2 = h + _B_ref(_layernorm(h, axis=-1), B_w_gate, B_w_up, B_w_down)
    return h2
```

```python
import jax, jax.numpy as jnp
from jax import lax
from jax.experimental import pallas as pl
from jax.experimental.pallas import tpu as pltpu

S, D, DF = 2048, 1024, 3584
H, DH, W, DIL = 32, 32, 8, 2
TM = 256
HM = 128
FC = 512
RB = 8
NST = 2
BAR = 0
PIN = 2
LNB = 16
NT = S // TM
NC = DF // FC
HALO = 16
SCALE = DH ** -0.5
LOG2E = 1.4426950408889634
MASK_RAW = -1e9 / SCALE
f32, bf16 = jnp.float32, jnp.bfloat16


def _ln(x):
    m = jnp.mean(x, axis=-1, keepdims=True)
    xc = x - m
    v = jnp.mean(xc * xc, axis=-1, keepdims=True)
    return xc * lax.rsqrt(v + 1e-5)


def _ln_list(ref, row0, n):
    out = []
    for r in range(0, n, LNB):
        x = ref[pl.ds(pl.multiple_of(row0 + r, LNB), LNB), :].astype(f32)
        out.append(_ln(x).astype(bf16))
    return out


def _ln_blocks(ref, row0, n):
    return jnp.concatenate(_ln_list(ref, row0, n), axis=0)


def _pin1(a, deps, never):
    if not deps:
        return a
    a32 = pltpu.bitcast(a, jnp.uint32)
    lane = lax.broadcasted_iota(jnp.int32, (8, 128), 1)
    nv = lane < never
    top = []
    for t in range(a.shape[1] // 128):
        x = a32[0:8, t * 128:(t + 1) * 128]
        if t < len(deps):
            d32 = pltpu.bitcast(deps[t], jnp.uint32)
            x = jnp.where(nv, d32[0:8, t * 128:(t + 1) * 128], x)
        top.append(x)
    return pltpu.bitcast(jnp.concatenate([jnp.concatenate(top, axis=1), a32[8:]], axis=0), bf16)


def _mm_pinned(lhs, wfn, nchunks, deps, never, first=1):
    outs = []
    k = nchunks - first
    per = -(-len(deps) // k)
    for c in range(nchunks):
        d = deps[(c - first) * per:(c - first + 1) * per] if c >= first else []
        outs.append(wfn(_pin1(lhs, d, never), c))
    return jnp.concatenate(outs, axis=1)


def _pin(a, b, never):
    R, C = a.shape
    nb = b.shape[0] // 16
    a32 = pltpu.bitcast(a, jnp.uint32)
    b32 = pltpu.bitcast(b, jnp.uint32)
    lane = lax.broadcasted_iota(jnp.int32, (8, 128), 1)
    nv = lane < never
    rows = []
    nrb = R // 16
    per = nb // nrb
    for r in range(nrb):
        tiles = []
        for t in range(C // 128):
            x = a32[r * 8:(r + 1) * 8, t * 128:(t + 1) * 128]
            if t < per:
                bi = r * per + t
                x = jnp.where(nv, b32[bi * 8:(bi + 1) * 8, t * 128:(t + 1) * 128], x)
            tiles.append(x)
        rows.append(jnp.concatenate(tiles, axis=1))
    return pltpu.bitcast(jnp.concatenate(rows, axis=0), bf16)


def _rowperm(w):
    C = w.shape[1]
    w32 = pltpu.bitcast(w, jnp.uint32)
    blk = [w32[a * 8:(a + 1) * 8, :] for a in range(64)]
    sub = lax.broadcasted_iota(jnp.int32, (8, C), 0)
    stages = [(4, 2), (2, 4), (1, 8)][:NST]
    for s, ab in stages:
        bit = (sub & s) != 0
        new = [None] * 64
        for a in range(64):
            if a & ab:
                continue
            A, B = blk[a], blk[a | ab]
            new[a] = jnp.where(bit, pltpu.roll(B, s, 0), A)
            new[a | ab] = jnp.where(bit, B, pltpu.roll(A, 8 - s, 0))
        blk = new
    out = [None] * 64
    for a in range(64):
        if NST == 2:
            ap = (a & 7) * 8 + (a >> 3)
        else:
            ap = (a & 7) * 8 + ((a >> 3) & 1) * 4 + (a >> 4)
        out[ap] = blk[a]
    return pltpu.bitcast(jnp.concatenate(out, axis=0), bf16)


def _head_reduce(p, lane):
    if NST == 2:
        p = p + jnp.where((lane & 1) != 0, pltpu.roll(p, 1, 1), pltpu.roll(p, 127, 1))
        p = p + jnp.where((lane & 2) != 0, pltpu.roll(p, 2, 1), pltpu.roll(p, 126, 1))
    else:
        p = p + pltpu.roll(p, 64, 1)
        p = p + jnp.where((lane & 1) != 0, pltpu.roll(p, 1, 1), pltpu.roll(p, 127, 1))
    return p


def _nt(a, b):
    return lax.dot_general(a, b, (((1,), (1,)), ((), ())), preferred_element_type=f32)


def _nn(a, b):
    return jnp.dot(a, b, preferred_element_type=f32)


def _softmax_part(q, kbuf, rb, n, row0_global, never):
    lane = lax.broadcasted_iota(jnp.int32, (n, 128), 1)
    qs = [q[:, j * 128:(j + 1) * 128] for j in range(8)]
    if BAR:
        nv = lane < never
        qs = [jnp.where(nv, qs[7], qs[j]) for j in range(7)] + [qs[7]]
    logits = []
    for w in range(W):
        base = HALO + rb - DIL * w
        p = qs[0] * kbuf[0, base:base + n, :]
        for j in range(1, 8):
            p = p + qs[j] * kbuf[j, base:base + n, :]
        p = _head_reduce(p, lane)
        if rb < HALO and w > 0:
            row = row0_global + rb + lax.broadcasted_iota(jnp.int32, (n, 128), 0)
            p = jnp.where(row >= DIL * w, p, MASK_RAW)
        logits.append(p)
    m = logits[0]
    for w in range(1, W):
        m = jnp.maximum(m, logits[w])
    es = [jnp.exp2((l - m) * (SCALE * LOG2E)) for l in logits]
    den = es[0]
    for w in range(1, W):
        den = den + es[w]
    inv = 1.0 / den
    return [e * inv for e in es]


def _av_part(ps, vbuf, rb, n, never):
    if BAR:
        lane = lax.broadcasted_iota(jnp.int32, (n, 128), 1)
        nv = lane < never
        last = vbuf[7, HALO + rb:HALO + rb + n, :]
        ps = [jnp.where(nv, last, p) for p in ps]
    os_ = []
    for j in range(8):
        acc = None
        for w in range(W):
            base = HALO + rb - DIL * w
            t = ps[w] * vbuf[j, base:base + n, :]
            acc = t if acc is None else acc + t
        os_.append(acc)
    return jnp.concatenate(os_, axis=1)


def _gelu_mul(g, u):
    c = 0.7978845608028654
    t = jnp.tanh(g * (c + (c * 0.044715) * (g * g)))
    return (0.5 * g * (1.0 + t) * u).astype(bf16)


def kernel(x_hbm, wqkv_hbm, wo_hbm, wg_hbm, wu_hbm, wd_hbm, o_ref,
           xbuf, wraw, wt, wg, wu, wd, xn_scr, kbuf, vbuf, hbuf, hn_scr, zero_smem, sems):
    s = pl.program_id(0)

    def cp_x(t):
        rows = pl.ds(pl.multiple_of(t * TM, TM), TM)
        return pltpu.make_async_copy(x_hbm.at[rows, :], xbuf.at[rows, :], sems.at[9 + t])

    def cp_w(j):
        return pltpu.make_async_copy(wqkv_hbm.at[:, pl.ds(pl.multiple_of(j * D, D), D)], wraw.at[j], sems.at[1 + j])

    def cp_wo():
        return pltpu.make_async_copy(wo_hbm, wraw.at[3], sems.at[4])

    def cp_ffn():
        return [pltpu.make_async_copy(wg_hbm, wg, sems.at[6]),
                pltpu.make_async_copy(wu_hbm, wu, sems.at[7]),
                pltpu.make_async_copy(wd_hbm, wd, sems.at[8])]

    def tile_rows(tile):
        return pl.ds(pl.multiple_of(tile * TM, TM), TM)

    @pl.when(s == 0)
    @jax.named_scope("prologue")
    def _prologue():
        zero_smem[0] = 0
        cp_x(0).start()
        for j in range(3):
            cp_w(j).start()
        cp_wo().start()
        for t in range(1, NT):
            cp_x(t).start()
        for c in cp_ffn():
            c.start()
        cp_x(0).wait()
        xn_scr[...] = _ln_blocks(xbuf, 0, TM)
        for t in range(8):
            kbuf[t, TM:TM + HALO, :] = jnp.zeros((HALO, 128), f32)
            vbuf[t, TM:TM + HALO, :] = jnp.zeros((HALO, 128), f32)

        def it(j, c):
            cp_w(j).wait()
            wt[j] = _rowperm(wraw[j].T)
            return c
        lax.fori_loop(0, 3, it, 0)
        cp_wo().wait()
        wt[3] = _rowperm(wraw[3])

    @pl.when(s < NT - 1)
    @jax.named_scope("waitx")
    def _wait_x():
        cp_x(s + 1).wait()

    @pl.when(s < NT)
    @jax.named_scope("A")
    def _A():
        never = zero_smem[0]
        for t in range(8):
            kbuf[t, 0:HALO, :] = kbuf[t, TM:TM + HALO, :]
            vbuf[t, 0:HALO, :] = vbuf[t, TM:TM + HALO, :]
        xn_list = _ln_list(xbuf, jnp.minimum(s + 1, NT - 1) * TM, TM)
        xn_next = jnp.concatenate(xn_list, axis=0)
        os_ = []
        for r0 in range(0, TM, HM):
            xn = xn_scr[r0:r0 + HM, :]
            if PIN == 2 and r0 == 0:
                k = _mm_pinned(xn, lambda l, c: _nt(l, wt[1, c * 128:(c + 1) * 128, :]), 8, xn_list[:14], never)
            else:
                k = _nt(xn, wt[1])
            for t in range(8):
                kbuf[t, HALO + r0:HALO + r0 + HM, :] = k[:, t * 128:(t + 1) * 128]
            xq = xn
            if PIN == 1 and r0 == 0:
                xq = _pin(xn, xn_next, never)
            if PIN == 2 and r0 == 0:
                xq = _pin1(xn, xn_list[14:], never)
            q = _nt(xq, wt[0])
            v = _nt(xn, wt[2])
            for t in range(8):
                vbuf[t, HALO + r0:HALO + r0 + HM, :] = v[:, t * 128:(t + 1) * 128]
            o = []
            for rb in range(r0, r0 + HM, 2 * RB):
                blk = []
                for r in (rb, rb + RB):
                    p = _softmax_part(q[r - r0:r - r0 + RB], kbuf, r, RB, s * TM, never)
                    blk.append(_av_part(p, vbuf, r, RB, never))
                o.append(jnp.concatenate(blk, axis=0).astype(bf16))
            os_.append(jnp.concatenate(o, axis=0))
        xn_scr[...] = xn_next
        for hh in range(TM // HM):
            rows = pl.ds(pl.multiple_of(s * TM + hh * HM, HM), HM)
            hbuf[rows, :] = xbuf[rows, :].astype(f32) + _nn(os_[hh], wt[3])

    @pl.when(s == NT - 1)
    @jax.named_scope("trans")
    def _trans():
        for c in cp_ffn():
            c.wait()
        hn_scr[...] = _ln_blocks(hbuf, 0, TM)

    @pl.when(s >= NT)
    @jax.named_scope("B")
    def _B():
        t = s - NT
        hn = hn_scr[...]
        hn_list = _ln_list(hbuf, jnp.minimum(t + 1, NT - 1) * TM, TM)
        hn_next = jnp.concatenate(hn_list, axis=0)
        never = zero_smem[0]
        acc = hbuf[tile_rows(t), :]
        for c in range(NC):
            cs = slice(c * FC, (c + 1) * FC)
            if PIN == 2 and c == 0:
                nq = FC // 128
                g = _mm_pinned(hn, lambda l, n: _nn(l, wg[:, n * 128:(n + 1) * 128]), nq, hn_list[:6], never)
                u = _mm_pinned(hn, lambda l, n: _nn(l, wu[:, n * 128:(n + 1) * 128]), nq, hn_list[6:14], never, first=0)
                a = _gelu_mul(g, u)
            elif PIN == 2 and c == 1:
                a = _gelu_mul(_nn(_pin1(hn, hn_list[14:], never), wg[:, cs]), _nn(hn, wu[:, cs]))
            else:
                hu = _pin(hn, hn_next, never) if (PIN == 1 and c == 0) else hn
                a = _gelu_mul(_nn(hn, wg[:, cs]), _nn(hu, wu[:, cs]))
            acc = acc + _nn(a, wd[cs, :])
        hn_scr[...] = hn_next
        o_ref[...] = acc.astype(bf16)


@jax.jit
def pallas_sequential_preLN__sliding_local_dilated__glu_gated_geglu__prompt_kernel(
        A_x, A_wqkv, A_wo, B_x, B_w_gate, B_w_up, B_w_down):
    x = A_x.reshape(S, D)
    anyspec = pl.BlockSpec(memory_space=pl.ANY)
    out = pl.pallas_call(
        kernel,
        grid=(2 * NT,),
        in_specs=[anyspec] * 6,
        out_specs=pl.BlockSpec((TM, D), lambda i: (jnp.maximum(i - NT, 0), 0)),
        out_shape=jax.ShapeDtypeStruct((S, D), bf16),
        scratch_shapes=[
            pltpu.VMEM((S, D), bf16),
            pltpu.VMEM((4, D, D), bf16),
            pltpu.VMEM((4, D, D), bf16),
            pltpu.VMEM((D, DF), bf16),
            pltpu.VMEM((D, DF), bf16),
            pltpu.VMEM((DF, D), bf16),
            pltpu.VMEM((TM, D), bf16),
            pltpu.VMEM((8, TM + HALO, 128), f32),
            pltpu.VMEM((8, TM + HALO, 128), f32),
            pltpu.VMEM((S, D), f32),
            pltpu.VMEM((TM, D), bf16),
            pltpu.SMEM((1,), jnp.int32),
            pltpu.SemaphoreType.DMA((9 + NT,)),
        ],
        compiler_params=pltpu.CompilerParams(
            vmem_limit_bytes=110 * 1024 * 1024, dimension_semantics=("arbitrary",)),
    )(x, A_wqkv, A_wo, B_w_gate, B_w_up, B_w_down)
    return out.reshape(1, S, D)
```

```python
import jax, jax.numpy as jnp
from jax import lax
from jax.experimental import pallas as pl
from jax.experimental.pallas import tpu as pltpu

S, D, DF = 2048, 1024, 3584
H, DH, W, DIL = 32, 32, 8, 2
TM = 256
HM = 128
NT = S // TM
RB = 8
LNB = 16
HALO = 16
KH = D // 2
DFH = DF // 2
SCALE = DH ** -0.5
LOG2E = 1.4426950408889634
MASK_RAW = -1e9 / SCALE
f32, bf16, u32 = jnp.float32, jnp.bfloat16, jnp.uint32

SKEW = (3, 3, 1, 1)
SPLITW = 0
WO0FIRST = 2
LN2A = 0
PSCHED = 0
MERGE45 = 0
LNCH = 0
STARTP = 1
STARTDIV = 4
ENDP = 1
ENDA = 7
BCH = [512] * 7

ITEMS = [(1, 0), (1, 1), (0, 0), (0, 1), (2, 0), (2, 1)]


def _b16(x32):
    return pltpu.bitcast(x32, bf16)


def _w32(x16):
    return pltpu.bitcast(x16, u32)


def _nt(a, b):
    return lax.dot_general(a, b, (((1,), (1,)), ((), ())), preferred_element_type=f32)


def _nn(a, b):
    return jnp.dot(a, b, preferred_element_type=f32)


def _ln(x):
    m = jnp.mean(x, axis=-1, keepdims=True)
    xc = x - m
    v = jnp.mean(xc * xc, axis=-1, keepdims=True)
    return xc * lax.rsqrt(v + 1e-5)


def _rows(ref, row0, n):
    if ref.dtype == u32:
        h0 = row0 // 2 if isinstance(row0, int) else lax.shift_right_logical(row0, 1)
        return _b16(ref[pl.ds(pl.multiple_of(h0, 8), n // 2), :]).astype(f32)
    return ref[pl.ds(pl.multiple_of(row0, LNB), n), :]


def _ln_list(ref, row0, n):
    return [_ln(_rows(ref, row0 + r, LNB)).astype(bf16) for r in range(0, n, LNB)]


def _pin1(a, deps, never):
    if not deps:
        return a
    a32 = _w32(a)
    nv = lax.broadcasted_iota(jnp.int32, (8, 128), 1) < never
    top = []
    for t in range(a.shape[1] // 128):
        x = a32[0:8, t * 128:(t + 1) * 128]
        if t < len(deps):
            x = jnp.where(nv, _w32(deps[t])[0:8, t * 128:(t + 1) * 128], x)
        top.append(x)
    return _b16(jnp.concatenate([jnp.concatenate(top, axis=1), a32[8:]], axis=0))


def _mm_pinned(lhs, wfn, nchunks, deps, never, first=1):
    outs = []
    per = -(-len(deps) // (nchunks - first)) if deps else 0
    for c in range(nchunks):
        d = deps[(c - first) * per:(c - first + 1) * per] if (c >= first and deps) else []
        outs.append(wfn(_pin1(lhs, d, never), c))
    return jnp.concatenate(outs, axis=1)


def _perm_stage(blk, idx, stage):
    C = blk[idx[0]].shape[1]
    if stage < 3:
        s, ab = ((4, 2), (2, 4), (1, 8))[stage]
        bit = (lax.broadcasted_iota(jnp.int32, (8, C), 0) & s) != 0
        for a in idx:
            if a & ab:
                continue
            A, B = blk[a], blk[a | ab]
            blk[a] = jnp.where(bit, pltpu.roll(B, s, 0), A)
            blk[a | ab] = jnp.where(bit, B, pltpu.roll(A, 8 - s, 0))
    else:
        for a in idx:
            if a & 16:
                continue
            A, B = blk[a], blk[a | 16]
            blk[a] = (A & jnp.uint32(0xFFFF)) | (B << 16)
            blk[a | 16] = (A >> 16) | (B & jnp.uint32(0xFFFF0000))


def _perm_dest(a):
    return (a & 7) * 8 + ((a >> 3) & 1) * 4 + ((a >> 4) & 1) * 2 + (a >> 5)


def _rowperm(w32):
    blk = [w32[a * 8:(a + 1) * 8, :] for a in range(64)]
    for stage in range(4):
        _perm_stage(blk, list(range(64)), stage)
    out = [None] * 64
    for a in range(64):
        out[_perm_dest(a)] = blk[a]
    return jnp.concatenate(out, axis=0)


def _interleave(main, side):
    for i, f in enumerate(main):
        f()
        for g in (side[i] if i < len(side) else []):
            g()
    for rest in side[len(main):]:
        for g in rest:
            g()


def _probs_steps(q_rows, kbuf, r0, nrows, row0_global, sink):
    nb = nrows // RB
    st = [dict() for _ in range(nb)]

    def s1(b):
        r = r0 + b * RB
        q = q_rows(r)
        ps = []
        for w in range(W):
            base = HALO + r - DIL * w
            p = q[0] * kbuf[0, base:base + RB, :]
            for j in range(1, 8):
                p = p + q[j] * kbuf[j, base:base + RB, :]
            ps.append(p)
        st[b]["p"] = ps
        st[b]["r"] = [pltpu.roll(p, 64, 1) for p in ps]

    def s2(b):
        ps = [p + r for p, r in zip(st[b]["p"], st[b]["r"])]
        st[b]["p"] = ps
        st[b]["r"] = [pltpu.roll(p, 32, 1) for p in ps]

    def s3(b):
        r = r0 + b * RB
        ls = [p + x for p, x in zip(st[b]["p"], st[b]["r"])]
        if r < HALO:
            row = row0_global + r + lax.broadcasted_iota(jnp.int32, (RB, 128), 0)
            ls = [ls[0]] + [jnp.where(row >= DIL * w, ls[w], MASK_RAW) for w in range(1, W)]
        m = ls[0]
        for w in range(1, W):
            m = jnp.maximum(m, ls[w])
        st[b]["e"] = [jnp.exp2((l - m) * (SCALE * LOG2E)) for l in ls]

    def s4(b):
        es = st[b]["e"]
        den = es[0]
        for w in range(1, W):
            den = den + es[w]
        st[b]["inv"] = 1.0 / den

    def s5(b):
        sink(b, [e * st[b]["inv"] for e in st[b]["e"]])

    stages = [s1, s2, s3, s4, s5]
    offs = [0]
    for sk in SKEW:
        offs.append(offs[-1] + sk)
    steps = []
    for t in range(nb + offs[-1]):
        def step(t=t):
            for si in reversed(range(5)):
                b = t - offs[si]
                if 0 <= b < nb:
                    stages[si](b)
        steps.append(step)
    return steps


def _probs(q_rows, kbuf, r0, row0_global):
    out = [None] * (HM // RB)

    def sink(b, ps):
        out[b] = ps
    for f in _probs_steps(q_rows, kbuf, r0, HM, row0_global, sink):
        f()
    return out


def _av_block(ps2, vbuf, r, never):
    halves = []
    for e in range(2):
        rr = r + e * RB
        nv = lax.broadcasted_iota(jnp.int32, (RB, 128), 1) < never
        last = vbuf[7, HALO + rr:HALO + rr + RB, :]
        ps = [jnp.where(nv, last, p) for p in ps2[e]]
        os_ = []
        for j in range(8):
            acc = None
            for w in range(W):
                base = HALO + rr - DIL * w
                t = ps[w] * vbuf[j, base:base + RB, :]
                acc = t if acc is None else acc + t
            os_.append(acc)
        halves.append(jnp.concatenate(os_, axis=1))
    return jnp.concatenate(halves, axis=0).astype(bf16)


def _av(ps, vbuf, r0, never):
    return [_av_block(ps[i:i + 2], vbuf, r0 + i * RB, never) for i in range(0, len(ps), 2)]


def _gelu_mul(g, u):
    c = 0.7978845608028654
    t = jnp.tanh(g * (c + (c * 0.044715) * (g * g)))
    return (0.5 * g * (1.0 + t) * u).astype(bf16)


def kernel(x_hbm, wqkv_hbm, wo_hbm, wg_hbm, wu_hbm, wd_hbm, o_hbm,
           obuf, xbuf, wraw, wo_raw, wta, wtb, wo_p, wg, wu, wd, xn_scr, qkv,
           hbuf, hn_scr, zero_smem, sems, osems):
    kbuf = qkv.at[1]
    vbuf = qkv.at[2]

    def tile_rows(t):
        return pl.ds(pl.multiple_of(t * TM, TM), TM)

    def cp_x(t):
        rows = pl.ds(pl.multiple_of(t * (TM // 2), TM // 2), TM // 2)
        return pltpu.make_async_copy(x_hbm.bitcast(u32).at[rows, :], xbuf.at[rows, :], sems.at[11 + t])

    def cp_w(m, kh):
        cols = pl.ds(pl.multiple_of(m * D, D), D)
        return pltpu.make_async_copy(wqkv_hbm.bitcast(u32).at[kh * KH // 2:(kh + 1) * KH // 2, cols], wraw.at[kh, m],
                                     sems.at[2 * m + kh])

    def cp_wo(h):
        cs = slice(h * KH, (h + 1) * KH)
        return pltpu.make_async_copy(wo_hbm.bitcast(u32).at[:, cs], wo_raw.at[:, cs], sems.at[6 + h])

    def cp_ffn():
        return [pltpu.make_async_copy(wg_hbm.bitcast(u32), wg, sems.at[8]),
                pltpu.make_async_copy(wu_hbm.bitcast(u32), wu, sems.at[9]),
                pltpu.make_async_copy(wd_hbm.bitcast(u32), wd, sems.at[10])]

    def cp_o(t):
        return pltpu.make_async_copy(obuf.at[tile_rows(t), :], o_hbm.at[tile_rows(t), :], osems.at[t])

    def wo_part(s, o0, o1, never, deps1=()):
        o0f = jnp.concatenate(o0, axis=0)
        o1f = jnp.concatenate(o1, axis=0)
        rows0 = pl.ds(pl.multiple_of(s * TM, HM), HM)
        rows1 = pl.ds(pl.multiple_of(s * TM + HM, HM), HM)
        wfn = lambda l, c: _nn(l, _b16(wo_p[:, c * 128:(c + 1) * 128]))
        a0 = _mm_pinned(o0f, wfn, 8, o1[:8 - WO0FIRST], never, first=WO0FIRST)
        hbuf[rows0, :] = _rows(xbuf, s * TM, HM) + a0
        a1 = _mm_pinned(o1f, wfn, 8, list(deps1), never)
        hbuf[rows1, :] = _rows(xbuf, s * TM + HM, HM) + a1

    def setup(m, kh, never, start=None):
        dst = (wta, wtb)[kh]
        blk = [None] * 64
        for c in range(8):
            r32 = wraw[kh, m, :, c * 128:(c + 1) * 128]
            raw = _b16(r32)
            if start is not None:
                nv = lax.broadcasted_iota(jnp.int32, (8, 128), 1) < never
                d = pltpu.bitcast(start(c), u32)
                parts = []
                for r in range(0, r32.shape[0], 64):
                    parts += [jnp.where(nv, d, r32[r:r + 8]), r32[r + 8:r + 64]]
                raw = _b16(jnp.concatenate(parts, axis=0))
            t32 = _w32(raw.T)
            for a in range(8):
                blk[c * 8 + a] = t32[a * 8:(a + 1) * 8, :]
        for h in range(2):
            idx = list(range(h * 32, h * 32 + 32))
            for stage in range(4):
                _perm_stage(blk, idx, stage)
            for a in idx:
                d = _perm_dest(a)
                dst[m, d * 8:(d + 1) * 8, :] = blk[a]
        return blk

    def region(m, kh, m_next, kh_next, never):
        wsrc = (wta, wtb)[kh]
        res = {}

        def tile(n, deps=()):
            lhs = xn_scr[:, kh * KH:(kh + 1) * KH]
            if deps:
                nv = lax.broadcasted_iota(jnp.int32, (8, 128), 1) < never
                rows = []
                for rr in range(lhs.shape[0] // 8):
                    tiles = []
                    for t in range(lhs.shape[1] // 128):
                        x = lhs[rr * 8:(rr + 1) * 8, t * 128:(t + 1) * 128]
                        k = rr * (lhs.shape[1] // 128) + t
                        if k < len(deps):
                            x = jnp.where(nv, deps[k][:, 0:128], x)
                        tiles.append(x)
                    rows.append(jnp.concatenate(tiles, axis=1))
                lhs = jnp.concatenate(rows, axis=0)
            r = _nt(_b16(lhs), _b16(wsrc[m, n * 64:(n + 1) * 64, :]))
            res[n] = r[0:8]
            if kh == 1:
                r = r + qkv[m, n, HALO:HALO + TM, :]
            qkv[m, n, HALO:HALO + TM, :] = r

        for n in range(7):
            tile(n)
        blk = setup(m_next, kh_next, never, lambda c: res[c // STARTDIV])
        tile(7, blk)

    @jax.named_scope("P")
    def _first():
        zero_smem[0] = 0
        never = zero_smem[0]
        cp_x(0).start()
        cp_w(0, 0).start()
        cp_x(0).wait()
        for c in ([cp_w(0, 1)] + [cp_w(m, kh) for m in (1, 2) for kh in (0, 1)] + [cp_wo(0), cp_wo(1)]
                  + [cp_x(t) for t in range(1, NT)] + cp_ffn()):
            c.start()
        xn_scr[...] = _w32(jnp.concatenate(_ln_list(xbuf, 0, TM), axis=0))
        for t in range(8):
            kbuf[t, 0:HALO, :] = jnp.zeros((HALO, 128), f32)
            vbuf[t, 0:HALO, :] = jnp.zeros((HALO, 128), f32)
        cp_w(0, 0).wait()
        setup(0, 0, never)

        def body(m, carry):
            never = zero_smem[0]
            cp_w(m, 1).wait()
            region(m, 0, m, 1, never)

            @pl.when(m < 2)
            def _():
                cp_w(m + 1, 0).wait()
            region(m, 1, jnp.minimum(m + 1, 2), 0, never)
            return carry
        with jax.named_scope("Ploop"):
            lax.fori_loop(0, 3, body, 0)

        cp_wo(0).wait()
        cp_wo(1).wait()
        cp_x(1).wait()
        never = zero_smem[0]

        def q_rows(r):
            return [qkv[0, t, HALO + r:HALO + r + RB, :] for t in range(8)]
        o0 = _av(_probs(q_rows, kbuf, 0, 0), vbuf, 0, never)
        for c in range(8):
            wo_p[:, c * 128:(c + 1) * 128] = _rowperm(wo_raw[:, c * 128:(c + 1) * 128])
        o1 = _av(_probs(q_rows, kbuf, HM, 0), vbuf, HM, never)
        xn_list = _ln_list(xbuf, TM, TM)
        wo_part(0, o0, o1, never, xn_list[:14])
        xn_scr[...] = _w32(jnp.concatenate(xn_list, axis=0))

    @jax.named_scope("A")
    def _attn(s, carry):
        @pl.when(s < NT - 1)
        def _():
            cp_x(s + 1).wait()
        never = zero_smem[0]
        for t in range(8):
            kbuf[t, 0:HALO, :] = kbuf[t, TM:TM + HALO, :]
            vbuf[t, 0:HALO, :] = vbuf[t, TM:TM + HALO, :]
        xn_list = _ln_list(xbuf, jnp.minimum(s + 1, NT - 1) * TM, TM)

        def kqv(r0, kdeps, qdeps):
            xn = _b16(xn_scr[r0 // 2:(r0 + HM) // 2, :])
            def proj(l, m, rows=slice(None)):
                return _nt(l[:, 0:KH], _b16(wta[m, rows, :])) + _nt(l[:, KH:D], _b16(wtb[m, rows, :]))
            k = _mm_pinned(xn, lambda l, c: proj(l, 1, slice(c * 64, (c + 1) * 64)), 8, kdeps, never)
            for t in range(8):
                kbuf[t, HALO + r0:HALO + r0 + HM, :] = k[:, t * 128:(t + 1) * 128]
            q = proj(_pin1(xn, qdeps, never), 0)
            v = proj(xn, 2)
            for t in range(8):
                vbuf[t, HALO + r0:HALO + r0 + HM, :] = v[:, t * 128:(t + 1) * 128]
            return lambda r: [q[r - r0:r - r0 + RB, j * 128:(j + 1) * 128] for j in range(8)]

        q0 = kqv(0, xn_list[:14], xn_list[14:])
        o0 = _av(_probs(q0, kbuf, 0, s * TM), vbuf, 0, never)
        q1 = kqv(HM, o0[:7], o0[7:])
        o1 = _av(_probs(q1, kbuf, HM, s * TM), vbuf, HM, never)
        xn_scr[...] = _w32(jnp.concatenate(xn_list, axis=0))
        wo_part(s, o0, o1, never)
        return carry

    @jax.named_scope("B")
    def _ffn(t, carry):
        never = zero_smem[0]
        hn = _b16(hn_scr[...])
        hn_list = _ln_list(hbuf, jnp.minimum(t + 1, NT - 1) * TM, TM)
        acc = hbuf[tile_rows(t), :]
        off = 0
        for ci, fc in enumerate(BCH):
            cs = slice(off, off + fc)
            nq = fc // 128
            if ci == 0:
                g = _mm_pinned(hn, lambda l, n: _nn(l, _b16(wg[:, n * 128:(n + 1) * 128])), nq, hn_list[:6], never)
                u = _mm_pinned(hn, lambda l, n: _nn(l, _b16(wu[:, n * 128:(n + 1) * 128])), nq, hn_list[6:14], never, first=0)
            elif ci == 1:
                g = _nn(_pin1(hn, hn_list[14:], never), _b16(wg[:, cs]))
                u = _nn(hn, _b16(wu[:, cs]))
            else:
                g = _nn(hn, _b16(wg[:, cs]))
                u = _nn(hn, _b16(wu[:, cs]))
            acc = acc + _nn(_gelu_mul(g, u), _b16(wd[off // 2:(off + fc) // 2, :]))
            off += fc
        hn_scr[...] = _w32(jnp.concatenate(hn_list, axis=0))
        obuf[tile_rows(t), :] = acc.astype(bf16)
        cp_o(t).start()
        return carry

    _first()
    lax.fori_loop(1, NT, _attn, 0)
    with jax.named_scope("trans"):
        for c in cp_ffn():
            c.wait()
        hn_scr[...] = _w32(jnp.concatenate(_ln_list(hbuf, 0, TM), axis=0))
    lax.fori_loop(0, NT, _ffn, 0)
    for t in range(NT):
        cp_o(t).wait()


@jax.jit
def pallas_sequential_preLN__sliding_local_dilated__glu_gated_geglu__prompt_kernel(
        A_x, A_wqkv, A_wo, B_x, B_w_gate, B_w_up, B_w_down):
    x = A_x.reshape(S, D)
    anyspec = pl.BlockSpec(memory_space=pl.ANY)
    out = pl.pallas_call(
        kernel,
        in_specs=[anyspec] * 6,
        out_specs=anyspec,
        out_shape=jax.ShapeDtypeStruct((S, D), bf16),
        scratch_shapes=[
            pltpu.VMEM((S, D), bf16),
            pltpu.VMEM((S // 2, D), u32),
            pltpu.VMEM((2, 3, KH // 2, D), u32),
            pltpu.VMEM((D // 2, D), u32),
            pltpu.VMEM((3, D // 2, KH), u32),
            pltpu.VMEM((3, D // 2, KH), u32),
            pltpu.VMEM((D // 2, D), u32),
            pltpu.VMEM((D // 2, DF), u32),
            pltpu.VMEM((D // 2, DF), u32),
            pltpu.VMEM((DF // 2, D), u32),
            pltpu.VMEM((TM // 2, D), u32),
            pltpu.VMEM((3, 8, TM + HALO, 128), f32),
            pltpu.VMEM((S, D), f32),
            pltpu.VMEM((TM // 2, D), u32),
            pltpu.SMEM((1,), jnp.int32),
            pltpu.SemaphoreType.DMA((11 + NT,)),
            pltpu.SemaphoreType.DMA((NT,)),
        ],
        compiler_params=pltpu.CompilerParams(vmem_limit_bytes=110 * 1024 * 1024),
    )(x, A_wqkv, A_wo, B_w_gate, B_w_up, B_w_down)
    return out.reshape(1, S, D)
```

```python
import jax, jax.numpy as jnp
from jax import lax
from jax.experimental import pallas as pl
from jax.experimental.pallas import tpu as pltpu

S, D, DF = 2048, 1024, 3584
H, DH, W, DIL = 32, 32, 8, 2
TM = 256
HM = 128
NT = S // TM
RB = 8
LNB = 16
HALO = 16
KH = D // 2
DFH = DF // 2
SCALE = DH ** -0.5
LOG2E = 1.4426950408889634
MASK_RAW = -1e9 / SCALE
f32, bf16, u32 = jnp.float32, jnp.bfloat16, jnp.uint32

SKEW = (3, 3, 1, 1)
SPLITW = 0
WO0FIRST = 2
LN2A = 0
PSCHED = 0
MERGE45 = 0
LNCH = 0
PINSTEP = 4
NOCSE = 1
LNAFTER = 6
OSPLIT = 2
FUSEAV = 1
STARTP = 1
STARTDIV = 4
ENDP = 1
ENDA = 7
BCH = [512] * 7

ITEMS = [(1, 0), (1, 1), (0, 0), (0, 1), (2, 0), (2, 1)]


def _b16(x32):
    return pltpu.bitcast(x32, bf16)


def _w32(x16):
    return pltpu.bitcast(x16, u32)


def _nt(a, b):
    return lax.dot_general(a, b, (((1,), (1,)), ((), ())), preferred_element_type=f32)


def _nn(a, b):
    return jnp.dot(a, b, preferred_element_type=f32)


def _ln(x):
    m = jnp.mean(x, axis=-1, keepdims=True)
    xc = x - m
    v = jnp.mean(xc * xc, axis=-1, keepdims=True)
    return xc * lax.rsqrt(v + 1e-5)


def _rows(ref, row0, n):
    if ref.dtype == u32:
        h0 = row0 // 2 if isinstance(row0, int) else lax.shift_right_logical(row0, 1)
        return _b16(ref[pl.ds(pl.multiple_of(h0, 8), n // 2), :]).astype(f32)
    return ref[pl.ds(pl.multiple_of(row0, LNB), n), :]


def _ln_list(ref, row0, n, after=None, never=None):
    out = []
    for i, r in enumerate(range(0, n, LNB)):
        x = _rows(ref, row0 + r, LNB)
        if after is not None:
            nv = lax.broadcasted_iota(jnp.int32, (8, 128), 1) < never
            top = jnp.concatenate([jnp.where(nv, after(i), x[0:8, 0:128]), x[0:8, 128:]], axis=1)
            x = jnp.concatenate([top, x[8:]], axis=0)
        out.append(_ln(x).astype(bf16))
    return out


def _pin1(a, deps, never):
    if not deps:
        return a
    a32 = _w32(a)
    nv = lax.broadcasted_iota(jnp.int32, (8, 128), 1) < never
    top = []
    for t in range(a.shape[1] // 128):
        x = a32[0:8, t * 128:(t + 1) * 128]
        if t < len(deps):
            x = jnp.where(nv, _w32(deps[t])[0:8, t * 128:(t + 1) * 128], x)
        top.append(x)
    return _b16(jnp.concatenate([jnp.concatenate(top, axis=1), a32[8:]], axis=0))


def _mm_pinned(lhs, wfn, nchunks, deps, never, first=1):
    outs = []
    per = -(-len(deps) // (nchunks - first)) if deps else 0
    for c in range(nchunks):
        d = deps[(c - first) * per:(c - first + 1) * per] if (c >= first and deps) else []
        outs.append(wfn(_pin1(lhs, d, never), c))
    return jnp.concatenate(outs, axis=1)


def _perm_stage(blk, idx, stage):
    C = blk[idx[0]].shape[1]
    if stage < 3:
        s, ab = ((4, 2), (2, 4), (1, 8))[stage]
        bit = (lax.broadcasted_iota(jnp.int32, (8, C), 0) & s) != 0
        for a in idx:
            if a & ab:
                continue
            A, B = blk[a], blk[a | ab]
            blk[a] = jnp.where(bit, pltpu.roll(B, s, 0), A)
            blk[a | ab] = jnp.where(bit, B, pltpu.roll(A, 8 - s, 0))
    else:
        for a in idx:
            if a & 16:
                continue
            A, B = blk[a], blk[a | 16]
            blk[a] = (A & jnp.uint32(0xFFFF)) | (B << 16)
            blk[a | 16] = (A >> 16) | (B & jnp.uint32(0xFFFF0000))


def _perm_dest(a):
    return (a & 7) * 8 + ((a >> 3) & 1) * 4 + ((a >> 4) & 1) * 2 + (a >> 5)


def _perm_units(blk, half, store):
    C = blk[32 * half].shape[1]
    for a0 in range(2):
        idx = [a for a in range(32 * half, 32 * half + 32) if (a & 1) == a0]
        for t in range(C // 128):
            u = {a: blk[a][:, t * 128:(t + 1) * 128] for a in idx}
            for stage in range(4):
                _perm_stage(u, idx, stage)
            for a in idx:
                store(_perm_dest(a), t, u[a])


def _rowperm_into(dst, src, c):
    for half in range(2):
        blk = {a: src[a * 8:(a + 1) * 8, c * 128:(c + 1) * 128] for a in range(32 * half, 32 * half + 32)}

        def store(d, t, val):
            dst[d * 8:(d + 1) * 8, c * 128:(c + 1) * 128] = val
        _perm_units(blk, half, store)


def _interleave(main, side):
    for i, f in enumerate(main):
        f()
        for g in (side[i] if i < len(side) else []):
            g()
    for rest in side[len(main):]:
        for g in rest:
            g()


def _shifted(buf, j, r, w, zero):
    base = HALO + r - DIL * w
    if w >= 4 and zero is not None:
        return buf[j, pl.ds(base + zero, RB), :]
    return buf[j, base:base + RB, :]


def _probs_steps(q_rows, kbuf, r0, nrows, row0_global, sink, zero=None):
    nb = nrows // RB
    st = [dict() for _ in range(nb)]

    def s1(b):
        r = r0 + b * RB
        q = q_rows(r)
        ps = []
        for w in range(W):
            p = q[0] * _shifted(kbuf, 0, r, w, zero)
            for j in range(1, 8):
                p = p + q[j] * _shifted(kbuf, j, r, w, zero)
            ps.append(p)
        st[b]["p"] = ps
        st[b]["r"] = [pltpu.roll(p, 64, 1) for p in ps]

    def s2(b):
        ps = [p + r for p, r in zip(st[b]["p"], st[b]["r"])]
        st[b]["p"] = ps
        st[b]["r"] = [pltpu.roll(p, 32, 1) for p in ps]

    def s3(b):
        r = r0 + b * RB
        ls = [p + x for p, x in zip(st[b]["p"], st[b]["r"])]
        if r < HALO:
            row = row0_global + r + lax.broadcasted_iota(jnp.int32, (RB, 128), 0)
            ls = [ls[0]] + [jnp.where(row >= DIL * w, ls[w], MASK_RAW) for w in range(1, W)]
        m = ls[0]
        for w in range(1, W):
            m = jnp.maximum(m, ls[w])
        st[b]["e"] = [jnp.exp2((l - m) * (SCALE * LOG2E)) for l in ls]

    def s4(b):
        es = st[b]["e"]
        den = es[0]
        for w in range(1, W):
            den = den + es[w]
        st[b]["inv"] = 1.0 / den

    def s5(b):
        sink(b, [e * st[b]["inv"] for e in st[b]["e"]])

    stages = [s1, s2, s3, s4, s5]
    offs = [0]
    for sk in SKEW:
        offs.append(offs[-1] + sk)
    steps = []
    for t in range(nb + offs[-1]):
        def step(t=t):
            for si in reversed(range(5)):
                b = t - offs[si]
                if 0 <= b < nb:
                    stages[si](b)
        steps.append(step)
    return steps


def _probs(q_rows, kbuf, r0, row0_global, zero=None):
    out = [None] * (HM // RB)

    def sink(b, ps):
        out[b] = ps
    for f in _probs_steps(q_rows, kbuf, r0, HM, row0_global, sink, zero):
        f()
    return out


def _av_block(ps2, vbuf, r, never, zero=None):
    halves = []
    for e in range(2):
        rr = r + e * RB
        ps = ps2[e]
        if never is not None:
            nv = lax.broadcasted_iota(jnp.int32, (RB, 128), 1) < never
            last = vbuf[7, HALO + rr:HALO + rr + RB, :]
            ps = [jnp.where(nv, last, p) for p in ps]
        os_ = []
        for j in range(8):
            acc = None
            for w in range(W):
                t = ps[w] * _shifted(vbuf, j, rr, w, zero)
                acc = t if acc is None else acc + t
            os_.append(acc)
        halves.append(jnp.concatenate(os_, axis=1))
    return jnp.concatenate(halves, axis=0).astype(bf16)


def _av(ps, vbuf, r0, never, zero=None):
    return [_av_block(ps[i:i + 2], vbuf, r0 + i * RB, never, zero) for i in range(0, len(ps), 2)]


def _attn_fused(q_rows, kbuf, vbuf, r0, row0_global, zero=None):
    halves = {}

    def sink(b, ps):
        rr = r0 + b * RB
        os_ = []
        for j in range(8):
            acc = None
            for w in range(W):
                t = ps[w] * _shifted(vbuf, j, rr, w, zero)
                acc = t if acc is None else acc + t
            os_.append(acc)
        halves[b] = jnp.concatenate(os_, axis=1)
    for f in _probs_steps(q_rows, kbuf, r0, HM, row0_global, sink, zero):
        f()
    return [jnp.concatenate([halves[b], halves[b + 1]], axis=0).astype(bf16) for b in range(0, HM // RB, 2)]


def _gelu_mul(g, u):
    c = 0.7978845608028654
    t = jnp.tanh(g * (c + (c * 0.044715) * (g * g)))
    return (0.5 * g * (1.0 + t) * u).astype(bf16)


def kernel(x_hbm, wqkv_hbm, wo_hbm, wg_hbm, wu_hbm, wd_hbm, o_hbm,
           obuf, xbuf, wraw, wo_raw, wta, wtb, wo_p, wg, wu, wd, xn_scr, qkv,
           hbuf, hn_scr, zero_smem, sems, osems):
    kbuf = qkv.at[1]
    vbuf = qkv.at[2]

    def tile_rows(t):
        return pl.ds(pl.multiple_of(t * TM, TM), TM)

    def cp_x(t):
        rows = pl.ds(pl.multiple_of(t * (TM // 2), TM // 2), TM // 2)
        return pltpu.make_async_copy(x_hbm.bitcast(u32).at[rows, :], xbuf.at[rows, :], sems.at[11 + t])

    def cp_w(m, kh):
        cols = pl.ds(pl.multiple_of(m * D, D), D)
        return pltpu.make_async_copy(wqkv_hbm.bitcast(u32).at[kh * KH // 2:(kh + 1) * KH // 2, cols], wraw.at[kh, m],
                                     sems.at[2 * m + kh])

    def cp_wo(h):
        cs = slice(h * KH, (h + 1) * KH)
        return pltpu.make_async_copy(wo_hbm.bitcast(u32).at[:, cs], wo_raw.at[:, cs], sems.at[6 + h])

    def cp_ffn():
        return [pltpu.make_async_copy(wg_hbm.bitcast(u32), wg, sems.at[8]),
                pltpu.make_async_copy(wu_hbm.bitcast(u32), wu, sems.at[9]),
                pltpu.make_async_copy(wd_hbm.bitcast(u32), wd, sems.at[10])]

    def cp_o(t, h):
        cs = slice(h * (D // OSPLIT), (h + 1) * (D // OSPLIT))
        return pltpu.make_async_copy(obuf.at[tile_rows(t), cs], o_hbm.at[tile_rows(t), cs], osems.at[OSPLIT * t + h])

    def wo_part(s, o0, o1, never, deps1=None):
        o0f = jnp.concatenate(o0, axis=0)
        o1f = jnp.concatenate(o1, axis=0)
        rows0 = pl.ds(pl.multiple_of(s * TM, HM), HM)
        rows1 = pl.ds(pl.multiple_of(s * TM + HM, HM), HM)
        wfn = lambda l, c: _nn(l, _b16(wo_p[:, c * 128:(c + 1) * 128]))
        a0 = _mm_pinned(o0f, wfn, 8, o1[:8 - WO0FIRST], never, first=WO0FIRST)
        hbuf[rows0, :] = _rows(xbuf, s * TM, HM) + a0
        deps1 = deps1(a0) if deps1 is not None else []
        a1 = _mm_pinned(o1f, wfn, 8, deps1[:14], never)
        hbuf[rows1, :] = _rows(xbuf, s * TM + HM, HM) + a1
        return deps1

    def setup(m, kh, never, start=None):
        dst = (wta, wtb)[kh]
        blk = [None] * 64
        for c in range(8):
            r32 = wraw[kh, m, :, c * 128:(c + 1) * 128]
            raw = _b16(r32)
            if start is not None:
                nv = lax.broadcasted_iota(jnp.int32, (8, 128), 1) < never
                d = pltpu.bitcast(start(c), u32)
                parts = []
                for r in range(0, r32.shape[0], 64):
                    parts += [jnp.where(nv, d, r32[r:r + 8]), r32[r + 8:r + 64]]
                raw = _b16(jnp.concatenate(parts, axis=0))
            t32 = _w32(raw.T)
            for a in range(8):
                blk[c * 8 + a] = t32[a * 8:(a + 1) * 8, :]
        done = []

        def store(d, t, val):
            dst[m, d * 8:(d + 1) * 8, t * 128:(t + 1) * 128] = val
            done.append(val)
        for h in range(2):
            _perm_units(blk, h, store)
        return done[PINSTEP - 1::PINSTEP]

    def region(m, kh, m_next, kh_next, never):
        wsrc = (wta, wtb)[kh]
        res = {}

        def tile(n, deps=()):
            lhs = xn_scr[:, kh * KH:(kh + 1) * KH]
            if deps:
                nv = lax.broadcasted_iota(jnp.int32, (8, 128), 1) < never
                rows = []
                for rr in range(lhs.shape[0] // 8):
                    tiles = []
                    for t in range(lhs.shape[1] // 128):
                        x = lhs[rr * 8:(rr + 1) * 8, t * 128:(t + 1) * 128]
                        k = rr * (lhs.shape[1] // 128) + t
                        if k < len(deps):
                            x = jnp.where(nv, deps[k][:, 0:128], x)
                        tiles.append(x)
                    rows.append(jnp.concatenate(tiles, axis=1))
                lhs = jnp.concatenate(rows, axis=0)
            r = _nt(_b16(lhs), _b16(wsrc[m, n * 64:(n + 1) * 64, :]))
            res[n] = r[0:8]
            if kh == 1:
                r = r + qkv[m, n, HALO:HALO + TM, :]
            qkv[m, n, HALO:HALO + TM, :] = r

        for n in range(7):
            tile(n)
        blk = setup(m_next, kh_next, never, lambda c: res[c // STARTDIV])
        tile(7, blk)

    @jax.named_scope("P")
    def _first():
        zero_smem[0] = 0
        never = zero_smem[0]
        cp_x(0).start()
        cp_w(0, 0).start()
        cp_x(0).wait()
        for c in ([cp_w(0, 1)] + [cp_w(m, kh) for m in (1, 2) for kh in (0, 1)] + [cp_wo(0), cp_wo(1)]
                  + [cp_x(t) for t in range(1, NT)] + cp_ffn()):
            c.start()
        xn_scr[...] = _w32(jnp.concatenate(_ln_list(xbuf, 0, TM), axis=0))
        for t in range(8):
            kbuf[t, 0:HALO, :] = jnp.zeros((HALO, 128), f32)
            vbuf[t, 0:HALO, :] = jnp.zeros((HALO, 128), f32)
        cp_w(0, 0).wait()
        setup(0, 0, never)

        def body(m, carry):
            never = zero_smem[0]
            cp_w(m, 1).wait()
            region(m, 0, m, 1, never)

            @pl.when(m < 2)
            def _():
                cp_w(m + 1, 0).wait()
            region(m, 1, jnp.minimum(m + 1, 2), 0, never)
            return carry
        with jax.named_scope("Ploop"):
            lax.fori_loop(0, 3, body, 0)

        cp_wo(0).wait()
        cp_wo(1).wait()
        cp_x(1).wait()
        never = zero_smem[0]

        def q_rows(r):
            return [qkv[0, t, HALO + r:HALO + r + RB, :] for t in range(8)]
        o0 = _attn_fused(q_rows, kbuf, vbuf, 0, 0, never if NOCSE & 1 else None) if FUSEAV else _av(_probs(q_rows, kbuf, 0, 0), vbuf, 0, None)
        for c in range(8):
            _rowperm_into(wo_p, wo_raw, c)
        o1 = _attn_fused(q_rows, kbuf, vbuf, HM, 0, never if NOCSE & 1 else None) if FUSEAV else _av(_probs(q_rows, kbuf, HM, 0), vbuf, HM, None)
        xn_list = wo_part(0, o0, o1, never, lambda a0: _ln_list(
            xbuf, TM, TM, (lambda i: a0[0:8, LNAFTER * 128:(LNAFTER + 1) * 128]) if LNAFTER >= 0 else None, never))
        xn_scr[...] = _w32(jnp.concatenate(xn_list, axis=0))

    @jax.named_scope("A")
    def _attn(s, carry):
        @pl.when(s < NT - 1)
        def _():
            cp_x(s + 1).wait()
        never = zero_smem[0]
        for t in range(8):
            kbuf[t, 0:HALO, :] = kbuf[t, TM:TM + HALO, :]
            vbuf[t, 0:HALO, :] = vbuf[t, TM:TM + HALO, :]
        xn_list = _ln_list(xbuf, jnp.minimum(s + 1, NT - 1) * TM, TM)

        def kqv(r0, kdeps, qdeps):
            xn = _b16(xn_scr[r0 // 2:(r0 + HM) // 2, :])
            def proj(l, m, rows=slice(None)):
                return _nt(l[:, 0:KH], _b16(wta[m, rows, :])) + _nt(l[:, KH:D], _b16(wtb[m, rows, :]))
            k = _mm_pinned(xn, lambda l, c: proj(l, 1, slice(c * 64, (c + 1) * 64)), 8, kdeps, never)
            for t in range(8):
                kbuf[t, HALO + r0:HALO + r0 + HM, :] = k[:, t * 128:(t + 1) * 128]
            q = proj(_pin1(xn, qdeps, never), 0)
            v = proj(xn, 2)
            for t in range(8):
                vbuf[t, HALO + r0:HALO + r0 + HM, :] = v[:, t * 128:(t + 1) * 128]
            return lambda r: [q[r - r0:r - r0 + RB, j * 128:(j + 1) * 128] for j in range(8)]

        q0 = kqv(0, xn_list[:14], xn_list[14:])
        zk = never if NOCSE & 2 else None
        zv = never if NOCSE & 4 else None
        o0 = _av(_probs(q0, kbuf, 0, s * TM, zk), vbuf, 0, never, zv)
        q1 = kqv(HM, o0[:7], o0[7:])
        o1 = _av(_probs(q1, kbuf, HM, s * TM, zk), vbuf, HM, never, zv)
        xn_scr[...] = _w32(jnp.concatenate(xn_list, axis=0))
        nper = -(-(TM // LNB) // (NT - 1))
        blks = [jnp.minimum((s - 1) * nper + i, TM // LNB - 1) for i in range(nper)]
        hn_part = [_ln_list(hbuf, b * LNB, LNB)[0] for b in blks]
        wo_part(s, o0, o1, never, lambda a0: hn_part)
        for b, v in zip(blks, hn_part):
            hn_scr[pl.ds(pl.multiple_of(b * (LNB // 2), LNB // 2), LNB // 2), :] = _w32(v)
        return carry

    @jax.named_scope("B")
    def _ffn(t, carry):
        never = zero_smem[0]
        hn = _b16(hn_scr[...])
        hn_list = _ln_list(hbuf, jnp.minimum(t + 1, NT - 1) * TM, TM)
        acc = hbuf[tile_rows(t), :]
        off = 0
        for ci, fc in enumerate(BCH):
            cs = slice(off, off + fc)
            nq = fc // 128
            if ci == 0:
                g = _mm_pinned(hn, lambda l, n: _nn(l, _b16(wg[:, n * 128:(n + 1) * 128])), nq, hn_list[:6], never)
                u = _mm_pinned(hn, lambda l, n: _nn(l, _b16(wu[:, n * 128:(n + 1) * 128])), nq, hn_list[6:14], never, first=0)
            elif ci == 1:
                g = _nn(_pin1(hn, hn_list[14:], never), _b16(wg[:, cs]))
                u = _nn(hn, _b16(wu[:, cs]))
            else:
                g = _nn(hn, _b16(wg[:, cs]))
                u = _nn(hn, _b16(wu[:, cs]))
            a = _gelu_mul(g, u)
            if ci < len(BCH) - 1:
                acc = acc + _nn(a, _b16(wd[off // 2:(off + fc) // 2, :]))
            else:
                hn_scr[...] = _w32(jnp.concatenate(hn_list, axis=0))
                for h in range(OSPLIT):
                    cs = slice(h * (D // OSPLIT), (h + 1) * (D // OSPLIT))
                    out = acc[:, cs] + _nn(a, _b16(wd[off // 2:(off + fc) // 2, cs]))
                    obuf[tile_rows(t), cs] = out.astype(bf16)
                    cp_o(t, h).start()
            off += fc
        return carry

    _first()
    lax.fori_loop(1, NT, _attn, 0)
    with jax.named_scope("trans"):
        for c in cp_ffn():
            c.wait()
    lax.fori_loop(0, NT, _ffn, 0)
    for t in range(NT):
        for h in range(OSPLIT):
            cp_o(t, h).wait()


@jax.jit
def pallas_sequential_preLN__sliding_local_dilated__glu_gated_geglu__prompt_kernel(
        A_x, A_wqkv, A_wo, B_x, B_w_gate, B_w_up, B_w_down):
    x = A_x.reshape(S, D)
    anyspec = pl.BlockSpec(memory_space=pl.ANY)
    out = pl.pallas_call(
        kernel,
        in_specs=[anyspec] * 6,
        out_specs=anyspec,
        out_shape=jax.ShapeDtypeStruct((S, D), bf16),
        scratch_shapes=[
            pltpu.VMEM((S, D), bf16),
            pltpu.VMEM((S // 2, D), u32),
            pltpu.VMEM((2, 3, KH // 2, D), u32),
            pltpu.VMEM((D // 2, D), u32),
            pltpu.VMEM((3, D // 2, KH), u32),
            pltpu.VMEM((3, D // 2, KH), u32),
            pltpu.VMEM((D // 2, D), u32),
            pltpu.VMEM((D // 2, DF), u32),
            pltpu.VMEM((D // 2, DF), u32),
            pltpu.VMEM((DF // 2, D), u32),
            pltpu.VMEM((TM // 2, D), u32),
            pltpu.VMEM((3, 8, TM + HALO, 128), f32),
            pltpu.VMEM((S, D), f32),
            pltpu.VMEM((TM // 2, D), u32),
            pltpu.SMEM((1,), jnp.int32),
            pltpu.SemaphoreType.DMA((11 + NT,)),
            pltpu.SemaphoreType.DMA((OSPLIT * NT,)),
        ],
        compiler_params=pltpu.CompilerParams(vmem_limit_bytes=110 * 1024 * 1024),
    )(x, A_wqkv, A_wo, B_w_gate, B_w_up, B_w_down)
    return out.reshape(1, S, D)
```

```python
import jax, jax.numpy as jnp
from jax import lax
from jax.experimental import pallas as pl
from jax.experimental.pallas import tpu as pltpu

S, D, DF = 2048, 1024, 3584
H, DH, W, DIL = 32, 32, 8, 2
TM = 256
HM = 128
NT = S // TM
RB = 8
LNB = 16
HALO = 16
KH = D // 2
DFH = DF // 2
SCALE = DH ** -0.5
LOG2E = 1.4426950408889634
MASK_RAW = -1e9 / SCALE
f32, bf16, u32 = jnp.float32, jnp.bfloat16, jnp.uint32


SKEW = (3, 3, 1, 1)
SPLITW = 0
WO0FIRST = 2
LN2A = 0
PSCHED = 0
MERGE45 = 0
LNCH = 0
PINSTEP = 4
NOCSE = 1
LNAFTER = 6
OSPLIT = 2
FUSEAV = 1
STARTP = 1
STARTDIV = 4
ENDP = 1
ENDA = 7
BCH = [1024, 1024, 1024, 512]

ITEMS = [(1, 0), (1, 1), (0, 0), (0, 1), (2, 0), (2, 1)]


def _b16(x32):
    return pltpu.bitcast(x32, bf16)


def _w32(x16):
    return pltpu.bitcast(x16, u32)


def _nt(a, b):
    return lax.dot_general(a, b, (((1,), (1,)), ((), ())), preferred_element_type=f32)


def _nn(a, b):
    return jnp.dot(a, b, preferred_element_type=f32)


def _ln(x):
    m = jnp.mean(x, axis=-1, keepdims=True)
    xc = x - m
    v = jnp.mean(xc * xc, axis=-1, keepdims=True)
    return xc * lax.rsqrt(v + 1e-5)


def _rows(ref, row0, n):
    if ref.dtype == u32:
        h0 = row0 // 2 if isinstance(row0, int) else lax.shift_right_logical(row0, 1)
        return _b16(ref[pl.ds(pl.multiple_of(h0, 8), n // 2), :]).astype(f32)
    return ref[pl.ds(pl.multiple_of(row0, LNB), n), :]


def _ln_list(ref, row0, n, after=None, never=None):
    out = []
    for i, r in enumerate(range(0, n, LNB)):
        x = _rows(ref, row0 + r, LNB)
        if after is not None:
            nv = lax.broadcasted_iota(jnp.int32, (8, 128), 1) < never
            top = jnp.concatenate([jnp.where(nv, after(i), x[0:8, 0:128]), x[0:8, 128:]], axis=1)
            x = jnp.concatenate([top, x[8:]], axis=0)
        out.append(_ln(x).astype(bf16))
    return out


def _pin1(a, deps, never):
    if not deps:
        return a
    a32 = _w32(a)
    nv = lax.broadcasted_iota(jnp.int32, (8, 128), 1) < never
    top = []
    for t in range(a.shape[1] // 128):
        x = a32[0:8, t * 128:(t + 1) * 128]
        if t < len(deps):
            x = jnp.where(nv, _w32(deps[t])[0:8, t * 128:(t + 1) * 128], x)
        top.append(x)
    return _b16(jnp.concatenate([jnp.concatenate(top, axis=1), a32[8:]], axis=0))


def _mm_pinned(lhs, wfn, nchunks, deps, never, first=1):
    outs = []
    per = -(-len(deps) // (nchunks - first)) if deps else 0
    for c in range(nchunks):
        d = deps[(c - first) * per:(c - first + 1) * per] if (c >= first and deps) else []
        outs.append(wfn(_pin1(lhs, d, never), c))
    return jnp.concatenate(outs, axis=1)


def _perm_stage(blk, idx, stage):
    C = blk[idx[0]].shape[1]
    if stage < 3:
        s, ab = ((4, 2), (2, 4), (1, 8))[stage]
        bit = (lax.broadcasted_iota(jnp.int32, (8, C), 0) & s) != 0
        for a in idx:
            if a & ab:
                continue
            A, B = blk[a], blk[a | ab]
            blk[a] = jnp.where(bit, pltpu.roll(B, s, 0), A)
            blk[a | ab] = jnp.where(bit, B, pltpu.roll(A, 8 - s, 0))
    else:
        for a in idx:
            if a & 16:
                continue
            A, B = blk[a], blk[a | 16]
            blk[a] = (A & jnp.uint32(0xFFFF)) | (B << 16)
            blk[a | 16] = (A >> 16) | (B & jnp.uint32(0xFFFF0000))


def _perm_dest(a):
    return (a & 7) * 8 + ((a >> 3) & 1) * 4 + ((a >> 4) & 1) * 2 + (a >> 5)


def _perm_units(blk, half, store):
    C = blk[32 * half].shape[1]
    for a0 in range(2):
        idx = [a for a in range(32 * half, 32 * half + 32) if (a & 1) == a0]
        for t in range(C // 128):
            u = {a: blk[a][:, t * 128:(t + 1) * 128] for a in idx}
            for stage in range(4):
                _perm_stage(u, idx, stage)
            for a in idx:
                store(_perm_dest(a), t, u[a])


def _rowperm_into(dst, src, c):
    for half in range(2):
        blk = {a: src[a * 8:(a + 1) * 8, c * 128:(c + 1) * 128] for a in range(32 * half, 32 * half + 32)}

        def store(d, t, val):
            dst[d * 8:(d + 1) * 8, c * 128:(c + 1) * 128] = val
        _perm_units(blk, half, store)


def _interleave(main, side):
    for i, f in enumerate(main):
        f()
        for g in (side[i] if i < len(side) else []):
            g()
    for rest in side[len(main):]:
        for g in rest:
            g()


def _shifted(buf, j, r, w, zero):
    base = HALO + r - DIL * w
    if w >= 4 and zero is not None:
        return buf[j, pl.ds(base + zero, RB), :]
    return buf[j, base:base + RB, :]


def _probs_steps(q_rows, kbuf, r0, nrows, row0_global, sink, zero=None):
    nb = nrows // RB
    st = [dict() for _ in range(nb)]

    def s1(b):
        r = r0 + b * RB
        q = q_rows(r)
        ps = []
        for w in range(W):
            p = q[0] * _shifted(kbuf, 0, r, w, zero)
            for j in range(1, 8):
                p = p + q[j] * _shifted(kbuf, j, r, w, zero)
            ps.append(p)
        st[b]["p"] = ps
        st[b]["r"] = [pltpu.roll(p, 64, 1) for p in ps]

    def s2(b):
        ps = [p + r for p, r in zip(st[b]["p"], st[b]["r"])]
        st[b]["p"] = ps
        st[b]["r"] = [pltpu.roll(p, 32, 1) for p in ps]

    def s3(b):
        r = r0 + b * RB
        ls = [p + x for p, x in zip(st[b]["p"], st[b]["r"])]
        if r < HALO:
            row = row0_global + r + lax.broadcasted_iota(jnp.int32, (RB, 128), 0)
            ls = [ls[0]] + [jnp.where(row >= DIL * w, ls[w], MASK_RAW) for w in range(1, W)]
        m = ls[0]
        for w in range(1, W):
            m = jnp.maximum(m, ls[w])
        st[b]["e"] = [jnp.exp2((l - m) * (SCALE * LOG2E)) for l in ls]

    def s4(b):
        es = st[b]["e"]
        den = es[0]
        for w in range(1, W):
            den = den + es[w]
        st[b]["inv"] = 1.0 / den

    def s5(b):
        sink(b, [e * st[b]["inv"] for e in st[b]["e"]])

    stages = [s1, s2, s3, s4, s5]
    offs = [0]
    for sk in SKEW:
        offs.append(offs[-1] + sk)
    steps = []
    for t in range(nb + offs[-1]):
        def step(t=t):
            for si in reversed(range(5)):
                b = t - offs[si]
                if 0 <= b < nb:
                    stages[si](b)
        steps.append(step)
    return steps


def _probs(q_rows, kbuf, r0, row0_global, zero=None):
    out = [None] * (HM // RB)

    def sink(b, ps):
        out[b] = ps
    for f in _probs_steps(q_rows, kbuf, r0, HM, row0_global, sink, zero):
        f()
    return out


def _av_block(ps2, vbuf, r, never, zero=None):
    halves = []
    for e in range(2):
        rr = r + e * RB
        ps = ps2[e]
        if never is not None:
            nv = lax.broadcasted_iota(jnp.int32, (RB, 128), 1) < never
            last = vbuf[7, HALO + rr:HALO + rr + RB, :]
            ps = [jnp.where(nv, last, p) for p in ps]
        os_ = []
        for j in range(8):
            acc = None
            for w in range(W):
                t = ps[w] * _shifted(vbuf, j, rr, w, zero)
                acc = t if acc is None else acc + t
            os_.append(acc)
        halves.append(jnp.concatenate(os_, axis=1))
    return jnp.concatenate(halves, axis=0).astype(bf16)


def _av(ps, vbuf, r0, never, zero=None):
    return [_av_block(ps[i:i + 2], vbuf, r0 + i * RB, never, zero) for i in range(0, len(ps), 2)]


def _attn_fused(q_rows, kbuf, vbuf, r0, row0_global, zero=None):
    halves = {}

    def sink(b, ps):
        rr = r0 + b * RB
        os_ = []
        for j in range(8):
            acc = None
            for w in range(W):
                t = ps[w] * _shifted(vbuf, j, rr, w, zero)
                acc = t if acc is None else acc + t
            os_.append(acc)
        halves[b] = jnp.concatenate(os_, axis=1)
    for f in _probs_steps(q_rows, kbuf, r0, HM, row0_global, sink, zero):
        f()
    return [jnp.concatenate([halves[b], halves[b + 1]], axis=0).astype(bf16) for b in range(0, HM // RB, 2)]


def _gelu_mul(g, u):
    c = 0.7978845608028654
    t = jnp.tanh(g * (c + (c * 0.044715) * (g * g)))
    return (0.5 * g * (1.0 + t) * u).astype(bf16)


def kernel(x_hbm, wqkv_hbm, wo_hbm, wg_hbm, wu_hbm, wd_hbm, o_hbm,
           obuf, xbuf, wraw, wo_raw, wta, wtb, wo_p, wg, wu, wd, xn_scr, o0buf, pbuf, qkv,
           hbuf, hn_scr, zero_smem, sems, osem):
    kbuf = qkv.at[1]
    vbuf = qkv.at[2]

    def tile_rows(t):
        return pl.ds(pl.multiple_of(t * TM, TM), TM)

    def cp_x(t):
        rows = pl.ds(pl.multiple_of(t * (TM // 2), TM // 2), TM // 2)
        return pltpu.make_async_copy(x_hbm.bitcast(u32).at[rows, :], xbuf.at[rows, :], sems.at[11 + t])

    def cp_w(m, kh):
        cols = pl.ds(pl.multiple_of(m * D, D), D)
        return pltpu.make_async_copy(wqkv_hbm.bitcast(u32).at[kh * KH // 2:(kh + 1) * KH // 2, cols], wraw.at[kh, m],
                                     sems.at[2 * m + kh])

    def cp_wo(h):
        cs = slice(h * KH, (h + 1) * KH)
        return pltpu.make_async_copy(wo_hbm.bitcast(u32).at[:, cs], wo_raw.at[:, cs], sems.at[6 + h])

    def cp_ffn():
        return [pltpu.make_async_copy(wg_hbm.bitcast(u32), wg, sems.at[8]),
                pltpu.make_async_copy(wu_hbm.bitcast(u32), wu, sems.at[9]),
                pltpu.make_async_copy(wd_hbm.bitcast(u32), wd, sems.at[10])]

    def cp_o(t, h):
        cs = slice(h * (D // OSPLIT), (h + 1) * (D // OSPLIT))
        return pltpu.make_async_copy(obuf.at[tile_rows(t), cs], o_hbm.at[tile_rows(t), cs], osem)

    def wo_part(s, o0, o1, never, deps1=None):
        o0f = jnp.concatenate(o0, axis=0)
        o1f = jnp.concatenate(o1, axis=0)
        rows0 = pl.ds(pl.multiple_of(s * TM, HM), HM)
        rows1 = pl.ds(pl.multiple_of(s * TM + HM, HM), HM)
        wfn = lambda l, c: _nn(l, _b16(wo_p[:, c * 128:(c + 1) * 128]))
        a0 = _mm_pinned(o0f, wfn, 8, o1[:8 - WO0FIRST], never, first=WO0FIRST)
        hbuf[rows0, :] = _rows(xbuf, s * TM, HM) + a0
        deps1 = deps1(a0) if deps1 is not None else []
        a1 = _mm_pinned(o1f, wfn, 8, deps1[:14], never)
        hbuf[rows1, :] = _rows(xbuf, s * TM + HM, HM) + a1
        return deps1

    def setup(m, kh, never, start=None):
        dst = (wta, wtb)[kh]
        blk = [None] * 64
        for c in range(8):
            r32 = wraw[kh, m, :, c * 128:(c + 1) * 128]
            raw = _b16(r32)
            if start is not None:
                nv = lax.broadcasted_iota(jnp.int32, (8, 128), 1) < never
                d = pltpu.bitcast(start(c), u32)
                parts = []
                for r in range(0, r32.shape[0], 64):
                    parts += [jnp.where(nv, d, r32[r:r + 8]), r32[r + 8:r + 64]]
                raw = _b16(jnp.concatenate(parts, axis=0))
            t32 = _w32(raw.T)
            for a in range(8):
                blk[c * 8 + a] = t32[a * 8:(a + 1) * 8, :]
        done = []

        def store(d, t, val):
            dst[m, d * 8:(d + 1) * 8, t * 128:(t + 1) * 128] = val
            done.append(val)
        for h in range(2):
            _perm_units(blk, h, store)
        return done[PINSTEP - 1::PINSTEP]

    def region(m, kh, m_next, kh_next, never):
        wsrc = (wta, wtb)[kh]
        res = {}

        def tile(n, deps=()):
            lhs = xn_scr[:, kh * KH:(kh + 1) * KH]
            if deps:
                nv = lax.broadcasted_iota(jnp.int32, (8, 128), 1) < never
                rows = []
                for rr in range(lhs.shape[0] // 8):
                    tiles = []
                    for t in range(lhs.shape[1] // 128):
                        x = lhs[rr * 8:(rr + 1) * 8, t * 128:(t + 1) * 128]
                        k = rr * (lhs.shape[1] // 128) + t
                        if k < len(deps):
                            x = jnp.where(nv, deps[k][:, 0:128], x)
                        tiles.append(x)
                    rows.append(jnp.concatenate(tiles, axis=1))
                lhs = jnp.concatenate(rows, axis=0)
            r = _nt(_b16(lhs), _b16(wsrc[m, n * 64:(n + 1) * 64, :]))
            res[n] = r[0:8]
            if kh == 1:
                r = r + qkv[m, n, HALO:HALO + TM, :]
            qkv[m, n, HALO:HALO + TM, :] = r

        for n in range(7):
            tile(n)
        blk = setup(m_next, kh_next, never, lambda c: res[c // STARTDIV])
        tile(7, blk)

    @jax.named_scope("P")
    def _first():
        zero_smem[0] = 0
        never = zero_smem[0]
        cp_x(0).start()
        cp_w(0, 0).start()
        cp_x(0).wait()
        for c in ([cp_w(0, 1)] + [cp_w(m, kh) for m in (1, 2) for kh in (0, 1)] + [cp_wo(0), cp_wo(1)]
                  + [cp_x(t) for t in range(1, NT)] + cp_ffn()):
            c.start()
        def ln0(i, carry):
            r = i * 64
            xn_scr[pl.ds(pl.multiple_of(i * 32, 32), 32), :] = _w32(jnp.concatenate(_ln_list(xbuf, r, 64), axis=0))
            return carry
        lax.fori_loop(0, TM // 64, ln0, 0)
        for t in range(8):
            kbuf[t, 0:HALO, :] = jnp.zeros((HALO, 128), f32)
            vbuf[t, 0:HALO, :] = jnp.zeros((HALO, 128), f32)
        cp_w(0, 0).wait()

        def setup0(h, carry):
            blk = {}
            for c in range(4):
                t32 = _w32(_b16(wraw[0, 0, :, pl.ds(pl.multiple_of((4 * h + c) * 128, 128), 128)]).T)
                for a in range(8):
                    blk[c * 8 + a] = t32[a * 8:(a + 1) * 8, :]

            def store(d, t, val):
                wta[0, pl.ds(pl.multiple_of((d + h) * 8, 8), 8), t * 128:(t + 1) * 128] = val
            _perm_units(blk, 0, store)
            return carry
        lax.fori_loop(0, 2, setup0, 0)

        def body(m, carry):
            never = zero_smem[0]
            cp_w(m, 1).wait()
            region(m, 0, m, 1, never)
            cp_w(m + 1, 0).wait()
            region(m, 1, m + 1, 0, never)
            return carry
        with jax.named_scope("Ploop"):
            lax.fori_loop(0, 2, body, 0)

        never = zero_smem[0]

        def q_rows(r):
            return [qkv[0, t, HALO + r:HALO + r + RB, :] for t in range(8)]

        def probs_to_buf(r0):
            def sink(b, ps):
                for w in range(W):
                    pbuf[w, r0 + b * RB:r0 + (b + 1) * RB, :] = ps[w]
            for f in _probs_steps(q_rows, kbuf, r0, HM, 0, sink, None):
                f()

        def load_probs(r0):
            return [[pbuf[w, r:r + RB, :] for w in range(W)] for r in range(r0, r0 + HM, RB)]

        def v_half(r0):
            lhs = _b16(xn_scr[r0 // 2:(r0 + HM) // 2, KH:D])
            for n in range(8):
                r = _nt(lhs, _b16(wtb[2, n * 64:(n + 1) * 64, :]))
                vbuf[n, HALO + r0:HALO + r0 + HM, :] = r + vbuf[n, HALO + r0:HALO + r0 + HM, :]

        cp_w(2, 1).wait()
        with jax.named_scope("Rv0"):
            region(2, 0, 2, 1, never)
            probs_to_buf(0)
        cp_wo(0).wait()
        with jax.named_scope("Rv1"):
            v_half(0)
            v_half(HM)
            for c in range(4):
                _rowperm_into(wo_p, wo_raw, c)
            probs_to_buf(HM)
            o0buf[...] = _w32(jnp.concatenate(_av(load_probs(0), vbuf, 0, None, None), axis=0))
        cp_wo(1).wait()
        cp_x(1).wait()
        for c in range(4, 8):
            _rowperm_into(wo_p, wo_raw, c)
        o1 = _av(load_probs(HM), vbuf, HM, None, never)
        xn_list = wo_part(0, [_b16(o0buf[...])], o1, never, lambda a0: _ln_list(
            xbuf, TM, TM, (lambda i: a0[0:8, LNAFTER * 128:(LNAFTER + 1) * 128]) if LNAFTER >= 0 else None, never))
        xn_scr[...] = _w32(jnp.concatenate(xn_list, axis=0))

    @jax.named_scope("A")
    def _attn(s, carry):
        @pl.when(s < NT - 1)
        def _():
            cp_x(s + 1).wait()
        never = zero_smem[0]
        for t in range(8):
            kbuf[t, 0:HALO, :] = kbuf[t, TM:TM + HALO, :]
            vbuf[t, 0:HALO, :] = vbuf[t, TM:TM + HALO, :]
        xn_list = _ln_list(xbuf, jnp.minimum(s + 1, NT - 1) * TM, TM)

        def kqv(r0, kdeps, qdeps):
            xn = _b16(xn_scr[r0 // 2:(r0 + HM) // 2, :])
            def proj(l, m, rows=slice(None)):
                return _nt(l[:, 0:KH], _b16(wta[m, rows, :])) + _nt(l[:, KH:D], _b16(wtb[m, rows, :]))
            k = _mm_pinned(xn, lambda l, c: proj(l, 1, slice(c * 64, (c + 1) * 64)), 8, kdeps, never)
            for t in range(8):
                kbuf[t, HALO + r0:HALO + r0 + HM, :] = k[:, t * 128:(t + 1) * 128]
            q = proj(_pin1(xn, qdeps, never), 0)
            v = proj(xn, 2)
            for t in range(8):
                vbuf[t, HALO + r0:HALO + r0 + HM, :] = v[:, t * 128:(t + 1) * 128]
            return lambda r: [q[r - r0:r - r0 + RB, j * 128:(j + 1) * 128] for j in range(8)]

        q0 = kqv(0, xn_list[:14], xn_list[14:])
        zk = never if NOCSE & 2 else None
        zv = never if NOCSE & 4 else None
        o0 = _av(_probs(q0, kbuf, 0, s * TM, zk), vbuf, 0, never, zv)
        q1 = kqv(HM, o0[:7], o0[7:])
        o1 = _av(_probs(q1, kbuf, HM, s * TM, zk), vbuf, HM, never, zv)
        xn_scr[...] = _w32(jnp.concatenate(xn_list, axis=0))
        nper = -(-(TM // LNB) // (NT - 1))
        blks = [jnp.minimum((s - 1) * nper + i, TM // LNB - 1) for i in range(nper)]
        hn_part = [_ln_list(hbuf, b * LNB, LNB)[0] for b in blks]
        wo_part(s, o0, o1, never, lambda a0: hn_part)
        for b, v in zip(blks, hn_part):
            hn_scr[pl.ds(pl.multiple_of(b * (LNB // 2), LNB // 2), LNB // 2), :] = _w32(v)
        return carry

    @jax.named_scope("B")
    def _ffn(t, carry):
        never = zero_smem[0]
        hn = _b16(hn_scr[...])
        hn_list = _ln_list(hbuf, jnp.minimum(t + 1, NT - 1) * TM, TM)
        acc = hbuf[tile_rows(t), :]
        off = 0
        for ci, fc in enumerate(BCH):
            cs = slice(off, off + fc)
            nq = fc // 128
            if ci == 0:
                g = _mm_pinned(hn, lambda l, n: _nn(l, _b16(wg[:, n * 128:(n + 1) * 128])), nq, hn_list[:6], never)
                u = _mm_pinned(hn, lambda l, n: _nn(l, _b16(wu[:, n * 128:(n + 1) * 128])), nq, hn_list[6:14], never, first=0)
            elif ci == 1:
                g = _nn(_pin1(hn, hn_list[14:], never), _b16(wg[:, cs]))
                u = _nn(hn, _b16(wu[:, cs]))
            else:
                g = _nn(hn, _b16(wg[:, cs]))
                u = _nn(hn, _b16(wu[:, cs]))
            a = _gelu_mul(g, u)
            if ci < len(BCH) - 1:
                acc = acc + _nn(a, _b16(wd[off // 2:(off + fc) // 2, :]))
            else:
                hn_scr[...] = _w32(jnp.concatenate(hn_list, axis=0))
                for h in range(OSPLIT):
                    cs = slice(h * (D // OSPLIT), (h + 1) * (D // OSPLIT))
                    out = acc[:, cs] + _nn(a, _b16(wd[off // 2:(off + fc) // 2, cs]))
                    obuf[tile_rows(t), cs] = out.astype(bf16)
                    cp_o(t, h).start()
            off += fc
        return carry

    _first()
    lax.fori_loop(1, NT, _attn, 0)
    with jax.named_scope("trans"):
        for c in cp_ffn():
            c.wait()
    lax.fori_loop(0, NT, _ffn, 0)
    pltpu.make_async_copy(obuf, o_hbm, osem).wait()


@jax.jit
def pallas_sequential_preLN__sliding_local_dilated__glu_gated_geglu__prompt_kernel(
        A_x, A_wqkv, A_wo, B_x, B_w_gate, B_w_up, B_w_down):
    x = A_x.reshape(S, D)
    anyspec = pl.BlockSpec(memory_space=pl.ANY)
    out = pl.pallas_call(
        kernel,
        in_specs=[anyspec] * 6,
        out_specs=anyspec,
        out_shape=jax.ShapeDtypeStruct((S, D), bf16),
        scratch_shapes=[
            pltpu.VMEM((S, D), bf16),
            pltpu.VMEM((S // 2, D), u32),
            pltpu.VMEM((2, 3, KH // 2, D), u32),
            pltpu.VMEM((D // 2, D), u32),
            pltpu.VMEM((3, D // 2, KH), u32),
            pltpu.VMEM((3, D // 2, KH), u32),
            pltpu.VMEM((D // 2, D), u32),
            pltpu.VMEM((D // 2, DF), u32),
            pltpu.VMEM((D // 2, DF), u32),
            pltpu.VMEM((DF // 2, D), u32),
            pltpu.VMEM((TM // 2, D), u32),
            pltpu.VMEM((HM // 2, D), u32),
            pltpu.VMEM((W, TM, 128), f32),
            pltpu.VMEM((3, 8, TM + HALO, 128), f32),
            pltpu.VMEM((S, D), f32),
            pltpu.VMEM((TM // 2, D), u32),
            pltpu.SMEM((1,), jnp.int32),
            pltpu.SemaphoreType.DMA((11 + NT,)),
            pltpu.SemaphoreType.DMA,
        ],
        compiler_params=pltpu.CompilerParams(vmem_limit_bytes=110 * 1024 * 1024),
    )(x, A_wqkv, A_wo, B_w_gate, B_w_up, B_w_down)
    return out.reshape(1, S, D)
```

```python
import jax, jax.numpy as jnp
from jax import lax
from jax.experimental import pallas as pl
from jax.experimental.pallas import tpu as pltpu

S, D, DF = 2048, 1024, 3584
H, DH, W, DIL = 32, 32, 8, 2
TM = 256
HM = 128
NT = S // TM
RB = 8
LNB = 16
HALO = 16
KH = D // 2
DFH = DF // 2
SCALE = DH ** -0.5
LOG2E = 1.4426950408889634
MASK_RAW = -1e9 / SCALE
f32, bf16, u32 = jnp.float32, jnp.bfloat16, jnp.uint32


SKEW = (3, 3, 1, 1)
SPLITW = 0
WO0FIRST = 2
LN2A = 0
PSCHED = 0
MERGE45 = 0
LNCH = 0
PINSTEP = 4
NOCSE = 1
LNAFTER = 2
RVPIN = 3
RV0PIN = 1
OSPLIT = 2
FUSEAV = 1
STARTP = 1
STARTDIV = 4
ENDP = 1
ENDA = 7
BCH = [1024, 1024, 1024, 512]

ITEMS = [(1, 0), (1, 1), (0, 0), (0, 1), (2, 0), (2, 1)]


def _b16(x32):
    return pltpu.bitcast(x32, bf16)


def _w32(x16):
    return pltpu.bitcast(x16, u32)


def _nt(a, b):
    return lax.dot_general(a, b, (((1,), (1,)), ((), ())), preferred_element_type=f32)


def _nn(a, b):
    return jnp.dot(a, b, preferred_element_type=f32)


def _ln(x):
    m = jnp.mean(x, axis=-1, keepdims=True)
    xc = x - m
    v = jnp.mean(xc * xc, axis=-1, keepdims=True)
    return xc * lax.rsqrt(v + 1e-5)


def _rows(ref, row0, n):
    if ref.dtype == u32:
        h0 = row0 // 2 if isinstance(row0, int) else lax.shift_right_logical(row0, 1)
        return _b16(ref[pl.ds(pl.multiple_of(h0, 8), n // 2), :]).astype(f32)
    return ref[pl.ds(pl.multiple_of(row0, LNB), n), :]


def _ln_list(ref, row0, n, after=None, never=None):
    out = []
    for i, r in enumerate(range(0, n, LNB)):
        x = _rows(ref, row0 + r, LNB)
        if after is not None:
            nv = lax.broadcasted_iota(jnp.int32, (8, 128), 1) < never
            top = jnp.concatenate([jnp.where(nv, after(i), x[0:8, 0:128]), x[0:8, 128:]], axis=1)
            x = jnp.concatenate([top, x[8:]], axis=0)
        out.append(_ln(x).astype(bf16))
    return out


def _pin1(a, deps, never):
    if not deps:
        return a
    a32 = _w32(a)
    nv = lax.broadcasted_iota(jnp.int32, (8, 128), 1) < never
    top = []
    for t in range(a.shape[1] // 128):
        x = a32[0:8, t * 128:(t + 1) * 128]
        if t < len(deps):
            x = jnp.where(nv, _w32(deps[t])[0:8, t * 128:(t + 1) * 128], x)
        top.append(x)
    return _b16(jnp.concatenate([jnp.concatenate(top, axis=1), a32[8:]], axis=0))


def _mm_pinned(lhs, wfn, nchunks, deps, never, first=1):
    outs = []
    per = -(-len(deps) // (nchunks - first)) if deps else 0
    for c in range(nchunks):
        d = deps[(c - first) * per:(c - first + 1) * per] if (c >= first and deps) else []
        outs.append(wfn(_pin1(lhs, d, never), c))
    return jnp.concatenate(outs, axis=1)


def _perm_stage(blk, idx, stage):
    C = blk[idx[0]].shape[1]
    if stage < 3:
        s, ab = ((4, 2), (2, 4), (1, 8))[stage]
        bit = (lax.broadcasted_iota(jnp.int32, (8, C), 0) & s) != 0
        for a in idx:
            if a & ab:
                continue
            A, B = blk[a], blk[a | ab]
            blk[a] = jnp.where(bit, pltpu.roll(B, s, 0), A)
            blk[a | ab] = jnp.where(bit, B, pltpu.roll(A, 8 - s, 0))
    else:
        for a in idx:
            if a & 16:
                continue
            A, B = blk[a], blk[a | 16]
            blk[a] = (A & jnp.uint32(0xFFFF)) | (B << 16)
            blk[a | 16] = (A >> 16) | (B & jnp.uint32(0xFFFF0000))


def _perm_dest(a):
    return (a & 7) * 8 + ((a >> 3) & 1) * 4 + ((a >> 4) & 1) * 2 + (a >> 5)


def _perm_units(blk, half, store):
    C = blk[32 * half].shape[1]
    for a0 in range(2):
        idx = [a for a in range(32 * half, 32 * half + 32) if (a & 1) == a0]
        for t in range(C // 128):
            u = {a: blk[a][:, t * 128:(t + 1) * 128] for a in idx}
            for stage in range(4):
                _perm_stage(u, idx, stage)
            for a in idx:
                store(_perm_dest(a), t, u[a])


def _rowperm_into(dst, src, c):
    done = []
    for half in range(2):
        blk = {a: src[a * 8:(a + 1) * 8, c * 128:(c + 1) * 128] for a in range(32 * half, 32 * half + 32)}

        def store(d, t, val):
            dst[d * 8:(d + 1) * 8, c * 128:(c + 1) * 128] = val
            done.append(val)
        _perm_units(blk, half, store)
    return done[15::16]


def _interleave(main, side):
    for i, f in enumerate(main):
        f()
        for g in (side[i] if i < len(side) else []):
            g()
    for rest in side[len(main):]:
        for g in rest:
            g()


def _shifted(buf, j, r, w, zero):
    base = HALO + r - DIL * w
    if w >= 4 and zero is not None:
        return buf[j, pl.ds(base + zero, RB), :]
    return buf[j, base:base + RB, :]


def _probs_steps(q_rows, kbuf, r0, nrows, row0_global, sink, zero=None):
    nb = nrows // RB
    st = [dict() for _ in range(nb)]

    def s1(b):
        r = r0 + b * RB
        q = q_rows(r)
        ps = []
        for w in range(W):
            p = q[0] * _shifted(kbuf, 0, r, w, zero)
            for j in range(1, 8):
                p = p + q[j] * _shifted(kbuf, j, r, w, zero)
            ps.append(p)
        st[b]["p"] = ps
        st[b]["r"] = [pltpu.roll(p, 64, 1) for p in ps]

    def s2(b):
        ps = [p + r for p, r in zip(st[b]["p"], st[b]["r"])]
        st[b]["p"] = ps
        st[b]["r"] = [pltpu.roll(p, 32, 1) for p in ps]

    def s3(b):
        r = r0 + b * RB
        ls = [p + x for p, x in zip(st[b]["p"], st[b]["r"])]
        if r < HALO:
            row = row0_global + r + lax.broadcasted_iota(jnp.int32, (RB, 128), 0)
            ls = [ls[0]] + [jnp.where(row >= DIL * w, ls[w], MASK_RAW) for w in range(1, W)]
        m = ls[0]
        for w in range(1, W):
            m = jnp.maximum(m, ls[w])
        st[b]["e"] = [jnp.exp2((l - m) * (SCALE * LOG2E)) for l in ls]

    def s4(b):
        es = st[b]["e"]
        den = es[0]
        for w in range(1, W):
            den = den + es[w]
        st[b]["inv"] = 1.0 / den

    def s5(b):
        sink(b, [e * st[b]["inv"] for e in st[b]["e"]])

    stages = [s1, s2, s3, s4, s5]
    offs = [0]
    for sk in SKEW:
        offs.append(offs[-1] + sk)
    steps = []
    for t in range(nb + offs[-1]):
        def step(t=t):
            for si in reversed(range(5)):
                b = t - offs[si]
                if 0 <= b < nb:
                    stages[si](b)
        steps.append(step)
    return steps


def _probs(q_rows, kbuf, r0, row0_global, zero=None):
    out = [None] * (HM // RB)

    def sink(b, ps):
        out[b] = ps
    for f in _probs_steps(q_rows, kbuf, r0, HM, row0_global, sink, zero):
        f()
    return out


def _av_block(ps2, vbuf, r, never, zero=None):
    halves = []
    for e in range(2):
        rr = r + e * RB
        ps = ps2[e]
        if never is not None:
            nv = lax.broadcasted_iota(jnp.int32, (RB, 128), 1) < never
            last = vbuf[7, HALO + rr:HALO + rr + RB, :]
            ps = [jnp.where(nv, last, p) for p in ps]
        os_ = []
        for j in range(8):
            acc = None
            for w in range(W):
                t = ps[w] * _shifted(vbuf, j, rr, w, zero)
                acc = t if acc is None else acc + t
            os_.append(acc)
        halves.append(jnp.concatenate(os_, axis=1))
    return jnp.concatenate(halves, axis=0).astype(bf16)


def _av(ps, vbuf, r0, never, zero=None):
    return [_av_block(ps[i:i + 2], vbuf, r0 + i * RB, never, zero) for i in range(0, len(ps), 2)]


def _attn_fused(q_rows, kbuf, vbuf, r0, row0_global, zero=None):
    halves = {}

    def sink(b, ps):
        rr = r0 + b * RB
        os_ = []
        for j in range(8):
            acc = None
            for w in range(W):
                t = ps[w] * _shifted(vbuf, j, rr, w, zero)
                acc = t if acc is None else acc + t
            os_.append(acc)
        halves[b] = jnp.concatenate(os_, axis=1)
    for f in _probs_steps(q_rows, kbuf, r0, HM, row0_global, sink, zero):
        f()
    return [jnp.concatenate([halves[b], halves[b + 1]], axis=0).astype(bf16) for b in range(0, HM // RB, 2)]


def _gelu_mul(g, u):
    c = 0.7978845608028654
    t = jnp.tanh(g * (c + (c * 0.044715) * (g * g)))
    return (0.5 * g * (1.0 + t) * u).astype(bf16)


def kernel(x_hbm, wqkv_hbm, wo_hbm, wg_hbm, wu_hbm, wd_hbm, o_hbm,
           obuf, xbuf, wraw, wo_raw, wta, wtb, wo_p, wg, wu, wd, xn_scr, o0buf, pbuf, qkv,
           hbuf, hn_scr, zero_smem, sems, osem):
    kbuf = qkv.at[1]
    vbuf = qkv.at[2]

    def tile_rows(t):
        return pl.ds(pl.multiple_of(t * TM, TM), TM)

    def cp_x(t):
        rows = pl.ds(pl.multiple_of(t * (TM // 2), TM // 2), TM // 2)
        return pltpu.make_async_copy(x_hbm.bitcast(u32).at[rows, :], xbuf.at[rows, :], sems.at[11 + t])

    def cp_w(m, kh):
        cols = pl.ds(pl.multiple_of(m * D, D), D)
        return pltpu.make_async_copy(wqkv_hbm.bitcast(u32).at[kh * KH // 2:(kh + 1) * KH // 2, cols], wraw.at[kh, m],
                                     sems.at[2 * m + kh])

    def cp_wo(h):
        cs = slice(h * KH, (h + 1) * KH)
        return pltpu.make_async_copy(wo_hbm.bitcast(u32).at[:, cs], wo_raw.at[:, cs], sems.at[6 + h])

    def cp_ffn():
        return [pltpu.make_async_copy(wg_hbm.bitcast(u32), wg, sems.at[8]),
                pltpu.make_async_copy(wu_hbm.bitcast(u32), wu, sems.at[9]),
                pltpu.make_async_copy(wd_hbm.bitcast(u32), wd, sems.at[10])]

    def cp_o(t, h):
        cs = slice(h * (D // OSPLIT), (h + 1) * (D // OSPLIT))
        return pltpu.make_async_copy(obuf.at[tile_rows(t), cs], o_hbm.at[tile_rows(t), cs], osem)

    def wo_part(s, o0, o1, never, deps1=None):
        o0f = jnp.concatenate(o0, axis=0)
        o1f = jnp.concatenate(o1, axis=0)
        rows0 = pl.ds(pl.multiple_of(s * TM, HM), HM)
        rows1 = pl.ds(pl.multiple_of(s * TM + HM, HM), HM)
        wfn = lambda l, c: _nn(l, _b16(wo_p[:, c * 128:(c + 1) * 128]))
        a0 = _mm_pinned(o0f, wfn, 8, o1[:8 - WO0FIRST], never, first=WO0FIRST)
        hbuf[rows0, :] = _rows(xbuf, s * TM, HM) + a0
        deps1 = deps1(a0) if deps1 is not None else []
        a1 = _mm_pinned(o1f, wfn, 8, deps1[:14], never)
        hbuf[rows1, :] = _rows(xbuf, s * TM + HM, HM) + a1
        return deps1

    def setup(m, kh, never, start=None):
        dst = (wta, wtb)[kh]
        blk = [None] * 64
        for c in range(8):
            r32 = wraw[kh, m, :, c * 128:(c + 1) * 128]
            raw = _b16(r32)
            if start is not None:
                nv = lax.broadcasted_iota(jnp.int32, (8, 128), 1) < never
                d = pltpu.bitcast(start(c), u32)
                parts = []
                for r in range(0, r32.shape[0], 64):
                    parts += [jnp.where(nv, d, r32[r:r + 8]), r32[r + 8:r + 64]]
                raw = _b16(jnp.concatenate(parts, axis=0))
            t32 = _w32(raw.T)
            for a in range(8):
                blk[c * 8 + a] = t32[a * 8:(a + 1) * 8, :]
        done = []

        def store(d, t, val):
            dst[m, d * 8:(d + 1) * 8, t * 128:(t + 1) * 128] = val
            done.append(val)
        for h in range(2):
            _perm_units(blk, h, store)
        return done[PINSTEP - 1::PINSTEP]

    def region(m, kh, m_next, kh_next, never, extra=lambda n: []):
        wsrc = (wta, wtb)[kh]
        res = {}

        def tile(n, deps=()):
            lhs = xn_scr[:, kh * KH:(kh + 1) * KH]
            if deps:
                nv = lax.broadcasted_iota(jnp.int32, (8, 128), 1) < never
                rows = []
                for rr in range(lhs.shape[0] // 8):
                    tiles = []
                    for t in range(lhs.shape[1] // 128):
                        x = lhs[rr * 8:(rr + 1) * 8, t * 128:(t + 1) * 128]
                        k = rr * (lhs.shape[1] // 128) + t
                        if k < len(deps):
                            x = jnp.where(nv, deps[k][:, 0:128], x)
                        tiles.append(x)
                    rows.append(jnp.concatenate(tiles, axis=1))
                lhs = jnp.concatenate(rows, axis=0)
            r = _nt(_b16(lhs), _b16(wsrc[m, n * 64:(n + 1) * 64, :]))
            res[n] = r[0:8]
            if kh == 1:
                r = r + qkv[m, n, HALO:HALO + TM, :]
            qkv[m, n, HALO:HALO + TM, :] = r

        for n in range(7):
            tile(n, extra(n))
        blk = setup(m_next, kh_next, never, lambda c: res[c // STARTDIV])
        tile(7, blk)

    @jax.named_scope("P")
    def _first():
        zero_smem[0] = 0
        never = zero_smem[0]
        cp_x(0).start()
        cp_w(0, 0).start()
        cp_x(0).wait()
        for c in ([cp_w(0, 1)] + [cp_w(m, kh) for m in (1, 2) for kh in (0, 1)] + [cp_wo(0), cp_wo(1)]
                  + [cp_x(t) for t in range(1, NT)] + cp_ffn()):
            c.start()
        def ln0(i, carry):
            r = i * 64
            xn_scr[pl.ds(pl.multiple_of(i * 32, 32), 32), :] = _w32(jnp.concatenate(_ln_list(xbuf, r, 64), axis=0))
            return carry
        lax.fori_loop(0, TM // 64, ln0, 0)
        for t in range(8):
            kbuf[t, 0:HALO, :] = jnp.zeros((HALO, 128), f32)
            vbuf[t, 0:HALO, :] = jnp.zeros((HALO, 128), f32)
        cp_w(0, 0).wait()

        def setup0(h, carry):
            blk = {}
            for c in range(4):
                t32 = _w32(_b16(wraw[0, 0, :, pl.ds(pl.multiple_of((4 * h + c) * 128, 128), 128)]).T)
                for a in range(8):
                    blk[c * 8 + a] = t32[a * 8:(a + 1) * 8, :]

            def store(d, t, val):
                wta[0, pl.ds(pl.multiple_of((d + h) * 8, 8), 8), t * 128:(t + 1) * 128] = val
            _perm_units(blk, 0, store)
            return carry
        lax.fori_loop(0, 2, setup0, 0)

        def body(m, carry):
            never = zero_smem[0]
            cp_w(m, 1).wait()
            region(m, 0, m, 1, never)
            cp_w(m + 1, 0).wait()
            region(m, 1, m + 1, 0, never)
            return carry
        with jax.named_scope("Ploop"):
            lax.fori_loop(0, 2, body, 0)

        never = zero_smem[0]

        def q_rows(r):
            return [qkv[0, t, HALO + r:HALO + r + RB, :] for t in range(8)]

        def probs_to_buf(r0):
            done = []

            def sink(b, ps):
                for w in range(W):
                    pbuf[w, r0 + b * RB:r0 + (b + 1) * RB, :] = ps[w]
                done.append(pltpu.bitcast(ps[0], u32))
            for f in _probs_steps(q_rows, kbuf, r0, HM, 0, sink, None):
                f()
            return done

        def load_probs(r0):
            return [[pbuf[w, r:r + RB, :] for w in range(W)] for r in range(r0, r0 + HM, RB)]

        def v_half(r0, deps=lambda n: []):
            lhs32 = xn_scr[r0 // 2:(r0 + HM) // 2, KH:D]
            nv = lax.broadcasted_iota(jnp.int32, (8, 128), 1) < never
            for n in range(8):
                lhs = lhs32
                ds = deps(n)
                if ds:
                    top = [lhs32[0:8, t * 128:(t + 1) * 128] for t in range(4)]
                    for i, d in enumerate(ds):
                        top[i] = jnp.where(nv, d, top[i])
                    lhs = jnp.concatenate([jnp.concatenate(top, axis=1), lhs32[8:]], axis=0)
                r = _nt(_b16(lhs), _b16(wtb[2, n * 64:(n + 1) * 64, :]))
                vbuf[n, HALO + r0:HALO + r0 + HM, :] = r + vbuf[n, HALO + r0:HALO + r0 + HM, :]

        cp_w(2, 1).wait()
        with jax.named_scope("Rv0"):
            pd0 = probs_to_buf(0)
            lo = [0, 0, 0, 4, 8, 12, 16, 16] if RV0PIN == 1 else [0, 0, 3, 6, 9, 12, 16, 16]
            region(2, 0, 2, 1, never, (lambda n: pd0[lo[n]:lo[n + 1]]) if RV0PIN else (lambda n: []))
        cp_wo(0).wait()
        def wo_cols(o, c0, c1, deps, first):
            wfn = lambda l, c: _nn(l, _b16(wo_p[:, (c0 + c) * 128:(c0 + c + 1) * 128]))
            return _mm_pinned(o, wfn, c1 - c0, deps, never, first=first)

        with jax.named_scope("Rv1"):
            v_half(0)
            rp = [_rowperm_into(wo_p, wo_raw, c) for c in range(4)]
            pd = probs_to_buf(HM)
            v_half(HM, lambda n: ([pd[2 * n + 1]] if RVPIN & 1 else []) + (rp[n // 2][2 * (n % 2):2 * (n % 2) + 2] if RVPIN & 2 else []))
            o0buf[...] = _w32(jnp.concatenate(_av(load_probs(0), vbuf, 0, None, None), axis=0))
            hbuf[0:HM, 0:KH] = _rows(xbuf, 0, HM)[:, 0:KH] + wo_cols(_b16(o0buf[...]), 0, 4, [], 1)
        cp_wo(1).wait()
        cp_x(1).wait()
        for c in range(4, 8):
            _rowperm_into(wo_p, wo_raw, c)
        o1 = _av(load_probs(HM), vbuf, HM, None, never)
        a0 = wo_cols(_b16(o0buf[...]), 4, 8, o1[:6], 1)
        hbuf[0:HM, KH:D] = _rows(xbuf, 0, HM)[:, KH:D] + a0
        xn_list = _ln_list(xbuf, TM, TM, lambda i: a0[0:8, LNAFTER * 128:(LNAFTER + 1) * 128], never)
        a1 = wo_cols(jnp.concatenate(o1, axis=0), 0, 8, xn_list[:14], 1)
        hbuf[HM:TM, :] = _rows(xbuf, HM, HM) + a1
        xn_scr[...] = _w32(jnp.concatenate(xn_list, axis=0))

    @jax.named_scope("A")
    def _attn(s, carry):
        @pl.when(s < NT - 1)
        def _():
            cp_x(s + 1).wait()
        never = zero_smem[0]
        for t in range(8):
            kbuf[t, 0:HALO, :] = kbuf[t, TM:TM + HALO, :]
            vbuf[t, 0:HALO, :] = vbuf[t, TM:TM + HALO, :]
        xn_list = _ln_list(xbuf, jnp.minimum(s + 1, NT - 1) * TM, TM)

        def kqv(r0, kdeps, qdeps):
            xn = _b16(xn_scr[r0 // 2:(r0 + HM) // 2, :])
            def proj(l, m, rows=slice(None)):
                return _nt(l[:, 0:KH], _b16(wta[m, rows, :])) + _nt(l[:, KH:D], _b16(wtb[m, rows, :]))
            k = _mm_pinned(xn, lambda l, c: proj(l, 1, slice(c * 64, (c + 1) * 64)), 8, kdeps, never)
            for t in range(8):
                kbuf[t, HALO + r0:HALO + r0 + HM, :] = k[:, t * 128:(t + 1) * 128]
            q = proj(_pin1(xn, qdeps, never), 0)
            v = proj(xn, 2)
            for t in range(8):
                vbuf[t, HALO + r0:HALO + r0 + HM, :] = v[:, t * 128:(t + 1) * 128]
            return lambda r: [q[r - r0:r - r0 + RB, j * 128:(j + 1) * 128] for j in range(8)]

        q0 = kqv(0, xn_list[:14], xn_list[14:])
        zk = never if NOCSE & 2 else None
        zv = never if NOCSE & 4 else None
        o0 = _av(_probs(q0, kbuf, 0, s * TM, zk), vbuf, 0, never, zv)
        q1 = kqv(HM, o0[:7], o0[7:])
        o1 = _av(_probs(q1, kbuf, HM, s * TM, zk), vbuf, HM, never, zv)
        xn_scr[...] = _w32(jnp.concatenate(xn_list, axis=0))
        nper = -(-(TM // LNB) // (NT - 1))
        blks = [jnp.minimum((s - 1) * nper + i, TM // LNB - 1) for i in range(nper)]
        hn_part = [_ln_list(hbuf, b * LNB, LNB)[0] for b in blks]
        wo_part(s, o0, o1, never, lambda a0: hn_part)
        for b, v in zip(blks, hn_part):
            hn_scr[pl.ds(pl.multiple_of(b * (LNB // 2), LNB // 2), LNB // 2), :] = _w32(v)
        return carry

    @jax.named_scope("B")
    def _ffn(t, carry):
        never = zero_smem[0]
        hn = _b16(hn_scr[...])
        hn_list = _ln_list(hbuf, jnp.minimum(t + 1, NT - 1) * TM, TM)
        acc = hbuf[tile_rows(t), :]
        off = 0
        for ci, fc in enumerate(BCH):
            cs = slice(off, off + fc)
            nq = fc // 128
            if ci == 0:
                g = _mm_pinned(hn, lambda l, n: _nn(l, _b16(wg[:, n * 128:(n + 1) * 128])), nq, hn_list[:6], never)
                u = _mm_pinned(hn, lambda l, n: _nn(l, _b16(wu[:, n * 128:(n + 1) * 128])), nq, hn_list[6:14], never, first=0)
            elif ci == 1:
                g = _nn(_pin1(hn, hn_list[14:], never), _b16(wg[:, cs]))
                u = _nn(hn, _b16(wu[:, cs]))
            else:
                g = _nn(hn, _b16(wg[:, cs]))
                u = _nn(hn, _b16(wu[:, cs]))
            a = _gelu_mul(g, u)
            if ci < len(BCH) - 1:
                acc = acc + _nn(a, _b16(wd[off // 2:(off + fc) // 2, :]))
            else:
                hn_scr[...] = _w32(jnp.concatenate(hn_list, axis=0))
                for h in range(OSPLIT):
                    cs = slice(h * (D // OSPLIT), (h + 1) * (D // OSPLIT))
                    out = acc[:, cs] + _nn(a, _b16(wd[off // 2:(off + fc) // 2, cs]))
                    obuf[tile_rows(t), cs] = out.astype(bf16)
                    cp_o(t, h).start()
            off += fc
        return carry

    _first()
    lax.fori_loop(1, NT, _attn, 0)
    with jax.named_scope("trans"):
        for c in cp_ffn():
            c.wait()
    lax.fori_loop(0, NT, _ffn, 0)
    pltpu.make_async_copy(obuf, o_hbm, osem).wait()


@jax.jit
def pallas_sequential_preLN__sliding_local_dilated__glu_gated_geglu__prompt_kernel(
        A_x, A_wqkv, A_wo, B_x, B_w_gate, B_w_up, B_w_down):
    x = A_x.reshape(S, D)
    anyspec = pl.BlockSpec(memory_space=pl.ANY)
    out = pl.pallas_call(
        kernel,
        in_specs=[anyspec] * 6,
        out_specs=anyspec,
        out_shape=jax.ShapeDtypeStruct((S, D), bf16),
        scratch_shapes=[
            pltpu.VMEM((S, D), bf16),
            pltpu.VMEM((S // 2, D), u32),
            pltpu.VMEM((2, 3, KH // 2, D), u32),
            pltpu.VMEM((D // 2, D), u32),
            pltpu.VMEM((3, D // 2, KH), u32),
            pltpu.VMEM((3, D // 2, KH), u32),
            pltpu.VMEM((D // 2, D), u32),
            pltpu.VMEM((D // 2, DF), u32),
            pltpu.VMEM((D // 2, DF), u32),
            pltpu.VMEM((DF // 2, D), u32),
            pltpu.VMEM((TM // 2, D), u32),
            pltpu.VMEM((HM // 2, D), u32),
            pltpu.VMEM((W, TM, 128), f32),
            pltpu.VMEM((3, 8, TM + HALO, 128), f32),
            pltpu.VMEM((S, D), f32),
            pltpu.VMEM((TM // 2, D), u32),
            pltpu.SMEM((1,), jnp.int32),
            pltpu.SemaphoreType.DMA((11 + NT,)),
            pltpu.SemaphoreType.DMA,
        ],
        compiler_params=pltpu.CompilerParams(vmem_limit_bytes=110 * 1024 * 1024),
    )(x, A_wqkv, A_wo, B_w_gate, B_w_up, B_w_down)
    return out.reshape(1, S, D)
```

```python
import jax
import jax.numpy as jnp
from jax import lax
from jax.experimental import pallas as pl
from jax.experimental.pallas import tpu as pltpu

S, D, DF = 2048, 1024, 3584
DH, W, DIL = 32, 8, 2
TM = 256
HM = 128
NT = S // TM
RB = 8
LNB = 16
HALO = 16
KH = D // 2
SCALE = DH ** -0.5
LOG2E = 1.4426950408889634
MASK_RAW = -1e9 / SCALE
f32, bf16, u32 = jnp.float32, jnp.bfloat16, jnp.uint32

SKEW = (3, 3, 1, 1)
BCH = (1024, 1024, 1024, 512)
OCUTS = (0, 512, 896, 1024)


def _b16(x32):
    return pltpu.bitcast(x32, bf16)


def _w32(x16):
    return pltpu.bitcast(x16, u32)


def _nt(a, b):
    return lax.dot_general(a, b, (((1,), (1,)), ((), ())), preferred_element_type=f32)


def _nn(a, b):
    return jnp.dot(a, b, preferred_element_type=f32)


def _ln(x):
    m = jnp.mean(x, axis=-1, keepdims=True)
    xc = x - m
    v = jnp.mean(xc * xc, axis=-1, keepdims=True)
    return xc * lax.rsqrt(v + 1e-5)


def _rows(ref, row0, n):
    if ref.dtype == u32:
        h0 = row0 // 2 if isinstance(row0, int) else lax.shift_right_logical(row0, 1)
        return _b16(ref[pl.ds(pl.multiple_of(h0, 8), n // 2), :]).astype(f32)
    return ref[pl.ds(pl.multiple_of(row0, LNB), n), :]


def _ln_list(ref, row0, n, after=None, never=None):
    out = []
    for i, r in enumerate(range(0, n, LNB)):
        x = _rows(ref, row0 + r, LNB)
        if after is not None:
            nv = lax.broadcasted_iota(jnp.int32, (8, 128), 1) < never
            top = jnp.concatenate([jnp.where(nv, after(i), x[0:8, 0:128]), x[0:8, 128:]], axis=1)
            x = jnp.concatenate([top, x[8:]], axis=0)
        out.append(_ln(x).astype(bf16))
    return out


def _pin1(a, deps, never):
    if not deps:
        return a
    a32 = _w32(a)
    nv = lax.broadcasted_iota(jnp.int32, (8, 128), 1) < never
    top = []
    for t in range(a.shape[1] // 128):
        x = a32[0:8, t * 128:(t + 1) * 128]
        if t < len(deps):
            x = jnp.where(nv, _w32(deps[t])[0:8, t * 128:(t + 1) * 128], x)
        top.append(x)
    return _b16(jnp.concatenate([jnp.concatenate(top, axis=1), a32[8:]], axis=0))


def _mm_pinned(lhs, wfn, nchunks, deps, never, first=1):
    outs = []
    per = -(-len(deps) // (nchunks - first)) if deps else 0
    for c in range(nchunks):
        d = deps[(c - first) * per:(c - first + 1) * per] if (c >= first and deps) else []
        outs.append(wfn(_pin1(lhs, d, never), c))
    return jnp.concatenate(outs, axis=1)


def _perm_stage(blk, idx, stage):
    C = blk[idx[0]].shape[1]
    if stage < 3:
        s, ab = ((4, 2), (2, 4), (1, 8))[stage]
        bit = (lax.broadcasted_iota(jnp.int32, (8, C), 0) & s) != 0
        for a in idx:
            if a & ab:
                continue
            A, B = blk[a], blk[a | ab]
            blk[a] = jnp.where(bit, pltpu.roll(B, s, 0), A)
            blk[a | ab] = jnp.where(bit, B, pltpu.roll(A, 8 - s, 0))
    else:
        for a in idx:
            if a & 16:
                continue
            A, B = blk[a], blk[a | 16]
            blk[a] = (A & jnp.uint32(0xFFFF)) | (B << 16)
            blk[a | 16] = (A >> 16) | (B & jnp.uint32(0xFFFF0000))


def _perm_dest(a):
    return (a & 7) * 8 + ((a >> 3) & 1) * 4 + ((a >> 4) & 1) * 2 + (a >> 5)


def _perm_units(blk, half, store):
    C = blk[32 * half].shape[1]
    for a0 in range(2):
        idx = [a for a in range(32 * half, 32 * half + 32) if (a & 1) == a0]
        for t in range(C // 128):
            u = {a: blk[a][:, t * 128:(t + 1) * 128] for a in idx}
            for stage in range(4):
                _perm_stage(u, idx, stage)
            for a in idx:
                store(_perm_dest(a), t, u[a])


def _rowperm_into(dst, src, c):
    done = []
    for half in range(2):
        blk = {a: src[a * 8:(a + 1) * 8, c * 128:(c + 1) * 128] for a in range(32 * half, 32 * half + 32)}

        def store(d, t, val):
            dst[d * 8:(d + 1) * 8, c * 128:(c + 1) * 128] = val
            done.append(val)
        _perm_units(blk, half, store)
    return done[15::16]


def _shifted(buf, j, r, w, zero):
    base = HALO + r - DIL * w
    if w >= 4 and zero is not None:
        return buf[j, pl.ds(base + zero, RB), :]
    return buf[j, base:base + RB, :]


def _probs_steps(q_rows, kbuf, r0, nrows, row0_global, sink, zero=None):
    nb = nrows // RB
    st = [dict() for _ in range(nb)]

    def s1(b):
        r = r0 + b * RB
        q = q_rows(r)
        ps = []
        for w in range(W):
            p = q[0] * _shifted(kbuf, 0, r, w, zero)
            for j in range(1, 8):
                p = p + q[j] * _shifted(kbuf, j, r, w, zero)
            ps.append(p)
        st[b]["p"] = ps
        st[b]["r"] = [pltpu.roll(p, 64, 1) for p in ps]

    def s2(b):
        ps = [p + r for p, r in zip(st[b]["p"], st[b]["r"])]
        st[b]["p"] = ps
        st[b]["r"] = [pltpu.roll(p, 32, 1) for p in ps]

    def s3(b):
        r = r0 + b * RB
        ls = [p + x for p, x in zip(st[b]["p"], st[b]["r"])]
        if r < HALO:
            row = row0_global + r + lax.broadcasted_iota(jnp.int32, (RB, 128), 0)
            ls = [ls[0]] + [jnp.where(row >= DIL * w, ls[w], MASK_RAW) for w in range(1, W)]
        m = ls[0]
        for w in range(1, W):
            m = jnp.maximum(m, ls[w])
        st[b]["e"] = [jnp.exp2((l - m) * (SCALE * LOG2E)) for l in ls]

    def s4(b):
        es = st[b]["e"]
        den = es[0]
        for w in range(1, W):
            den = den + es[w]
        st[b]["inv"] = 1.0 / den

    def s5(b):
        sink(b, [e * st[b]["inv"] for e in st[b]["e"]])

    stages = [s1, s2, s3, s4, s5]
    offs = [0]
    for sk in SKEW:
        offs.append(offs[-1] + sk)
    steps = []
    for t in range(nb + offs[-1]):
        def step(t=t):
            for si in reversed(range(5)):
                b = t - offs[si]
                if 0 <= b < nb:
                    stages[si](b)
        steps.append(step)
    return steps


def _probs(q_rows, kbuf, r0, row0_global, zero=None):
    out = [None] * (HM // RB)

    def sink(b, ps):
        out[b] = ps
    for f in _probs_steps(q_rows, kbuf, r0, HM, row0_global, sink, zero):
        f()
    return out


def _av_block(ps2, vbuf, r, never, zero=None):
    halves = []
    for e in range(2):
        rr = r + e * RB
        ps = ps2[e]
        if never is not None:
            nv = lax.broadcasted_iota(jnp.int32, (RB, 128), 1) < never
            last = vbuf[7, HALO + rr:HALO + rr + RB, :]
            ps = [jnp.where(nv, last, p) for p in ps]
        os_ = []
        for j in range(8):
            acc = None
            for w in range(W):
                t = ps[w] * _shifted(vbuf, j, rr, w, zero)
                acc = t if acc is None else acc + t
            os_.append(acc)
        halves.append(jnp.concatenate(os_, axis=1))
    return jnp.concatenate(halves, axis=0).astype(bf16)


def _av(ps, vbuf, r0, never, zero=None):
    return [_av_block(ps[i:i + 2], vbuf, r0 + i * RB, never, zero) for i in range(0, len(ps), 2)]


def _gelu_mul(g, u):
    c = 0.7978845608028654
    t = jnp.tanh(g * (c + (c * 0.044715) * (g * g)))
    return (0.5 * g * (1.0 + t) * u).astype(bf16)


def kernel(x_hbm, wqkv_hbm, wo_hbm, wg_hbm, wu_hbm, wd_hbm, o_hbm,
           obuf, xbuf, wraw, wo_raw, wta, wtb, wo_p, wg, wu, wd, xn_scr, o0buf, pbuf, qkv,
           hbuf, hn_scr, zero_smem, sems, osem):
    kbuf = qkv.at[1]
    vbuf = qkv.at[2]

    def tile_rows(t):
        return pl.ds(pl.multiple_of(t * TM, TM), TM)

    def cp_x(t):
        rows = pl.ds(pl.multiple_of(t * (TM // 2), TM // 2), TM // 2)
        return pltpu.make_async_copy(x_hbm.bitcast(u32).at[rows, :], xbuf.at[rows, :], sems.at[11 + t])

    def cp_w(m, kh):
        cols = pl.ds(pl.multiple_of(m * D, D), D)
        return pltpu.make_async_copy(wqkv_hbm.bitcast(u32).at[kh * KH // 2:(kh + 1) * KH // 2, cols], wraw.at[kh, m],
                                     sems.at[2 * m + kh])

    def cp_wo(h):
        cs = slice(h * KH, (h + 1) * KH)
        return pltpu.make_async_copy(wo_hbm.bitcast(u32).at[:, cs], wo_raw.at[:, cs], sems.at[6 + h])

    def cp_ffn():
        return [pltpu.make_async_copy(wg_hbm.bitcast(u32), wg, sems.at[8]),
                pltpu.make_async_copy(wu_hbm.bitcast(u32), wu, sems.at[9]),
                pltpu.make_async_copy(wd_hbm.bitcast(u32), wd, sems.at[10])]

    def cp_o(t, h):
        cs = slice(OCUTS[h], OCUTS[h + 1])
        return pltpu.make_async_copy(obuf.at[tile_rows(t), cs], o_hbm.at[tile_rows(t), cs], osem)

    def wo_part(s, o0, o1, never, deps1=None):
        o0f = jnp.concatenate(o0, axis=0)
        o1f = jnp.concatenate(o1, axis=0)
        rows0 = pl.ds(pl.multiple_of(s * TM, HM), HM)
        rows1 = pl.ds(pl.multiple_of(s * TM + HM, HM), HM)
        wfn = lambda l, c: _nn(l, _b16(wo_p[:, c * 128:(c + 1) * 128]))
        a0 = _mm_pinned(o0f, wfn, 8, o1[:6], never, first=2)
        hbuf[rows0, :] = _rows(xbuf, s * TM, HM) + a0
        deps1 = deps1(a0) if deps1 is not None else []
        a1 = _mm_pinned(o1f, wfn, 8, deps1[:14], never)
        hbuf[rows1, :] = _rows(xbuf, s * TM + HM, HM) + a1
        return deps1

    def setup(m, kh, never, start=None):
        dst = (wta, wtb)[kh]
        blk = [None] * 64
        for c in range(8):
            r32 = wraw[kh, m, :, c * 128:(c + 1) * 128]
            raw = _b16(r32)
            if start is not None:
                nv = lax.broadcasted_iota(jnp.int32, (8, 128), 1) < never
                d = pltpu.bitcast(start(c), u32)
                parts = []
                for r in range(0, r32.shape[0], 64):
                    parts += [jnp.where(nv, d, r32[r:r + 8]), r32[r + 8:r + 64]]
                raw = _b16(jnp.concatenate(parts, axis=0))
            t32 = _w32(raw.T)
            for a in range(8):
                blk[c * 8 + a] = t32[a * 8:(a + 1) * 8, :]
        done = []

        def store(d, t, val):
            dst[m, d * 8:(d + 1) * 8, t * 128:(t + 1) * 128] = val
            done.append(val)
        for h in range(2):
            _perm_units(blk, h, store)
        return done[3::4]

    def region(m, kh, m_next, kh_next, never, extra=lambda n: []):
        wsrc = (wta, wtb)[kh]
        res = {}

        def tile(n, deps=()):
            lhs = xn_scr[:, kh * KH:(kh + 1) * KH]
            if deps:
                nv = lax.broadcasted_iota(jnp.int32, (8, 128), 1) < never
                rows = []
                for rr in range(lhs.shape[0] // 8):
                    tiles = []
                    for t in range(lhs.shape[1] // 128):
                        x = lhs[rr * 8:(rr + 1) * 8, t * 128:(t + 1) * 128]
                        k = rr * (lhs.shape[1] // 128) + t
                        if k < len(deps):
                            x = jnp.where(nv, deps[k][:, 0:128], x)
                        tiles.append(x)
                    rows.append(jnp.concatenate(tiles, axis=1))
                lhs = jnp.concatenate(rows, axis=0)
            r = _nt(_b16(lhs), _b16(wsrc[m, n * 64:(n + 1) * 64, :]))
            res[n] = r[0:8]
            if kh == 1:
                r = r + qkv[m, n, HALO:HALO + TM, :]
            qkv[m, n, HALO:HALO + TM, :] = r

        for n in range(7):
            tile(n, extra(n))
        blk = setup(m_next, kh_next, never, lambda c: res[c // 4])
        tile(7, blk)

    @jax.named_scope("P")
    def _first():
        zero_smem[0] = 0
        never = zero_smem[0]
        cp_x(0).start()
        cp_w(0, 0).start()
        cp_x(0).wait()
        for c in ([cp_w(0, 1)] + [cp_w(m, kh) for m in (1, 2) for kh in (0, 1)] + [cp_wo(0), cp_wo(1)]
                  + [cp_x(t) for t in range(1, NT)] + cp_ffn()):
            c.start()
        def ln0(i, carry):
            r = i * 64
            xn_scr[pl.ds(pl.multiple_of(i * 32, 32), 32), :] = _w32(jnp.concatenate(_ln_list(xbuf, r, 64), axis=0))
            return carry
        lax.fori_loop(0, TM // 64, ln0, 0)
        for t in range(8):
            kbuf[t, 0:HALO, :] = jnp.zeros((HALO, 128), f32)
            vbuf[t, 0:HALO, :] = jnp.zeros((HALO, 128), f32)
        cp_w(0, 0).wait()

        def setup0(h, carry):
            blk = {}
            for c in range(4):
                t32 = _w32(_b16(wraw[0, 0, :, pl.ds(pl.multiple_of((4 * h + c) * 128, 128), 128)]).T)
                for a in range(8):
                    blk[c * 8 + a] = t32[a * 8:(a + 1) * 8, :]

            def store(d, t, val):
                wta[0, pl.ds(pl.multiple_of((d + h) * 8, 8), 8), t * 128:(t + 1) * 128] = val
            _perm_units(blk, 0, store)
            return carry
        lax.fori_loop(0, 2, setup0, 0)

        def body(m, carry):
            never = zero_smem[0]
            cp_w(m, 1).wait()
            region(m, 0, m, 1, never)
            cp_w(m + 1, 0).wait()
            region(m, 1, m + 1, 0, never)
            return carry
        with jax.named_scope("Ploop"):
            lax.fori_loop(0, 2, body, 0)

        never = zero_smem[0]

        def q_rows(r):
            return [qkv[0, t, HALO + r:HALO + r + RB, :] for t in range(8)]

        def probs_to_buf(r0):
            done = []

            def sink(b, ps):
                for w in range(W):
                    pbuf[w, r0 + b * RB:r0 + (b + 1) * RB, :] = ps[w]
                done.append(pltpu.bitcast(ps[0], u32))
            for f in _probs_steps(q_rows, kbuf, r0, HM, 0, sink, None):
                f()
            return done

        def load_probs(r0):
            return [[pbuf[w, r:r + RB, :] for w in range(W)] for r in range(r0, r0 + HM, RB)]

        def v_half(r0, deps=lambda n: []):
            lhs32 = xn_scr[r0 // 2:(r0 + HM) // 2, KH:D]
            nv = lax.broadcasted_iota(jnp.int32, (8, 128), 1) < never
            for n in range(8):
                lhs = lhs32
                ds = deps(n)
                if ds:
                    top = [lhs32[0:8, t * 128:(t + 1) * 128] for t in range(4)]
                    for i, d in enumerate(ds):
                        top[i] = jnp.where(nv, d, top[i])
                    lhs = jnp.concatenate([jnp.concatenate(top, axis=1), lhs32[8:]], axis=0)
                r = _nt(_b16(lhs), _b16(wtb[2, n * 64:(n + 1) * 64, :]))
                vbuf[n, HALO + r0:HALO + r0 + HM, :] = r + vbuf[n, HALO + r0:HALO + r0 + HM, :]

        cp_w(2, 1).wait()
        with jax.named_scope("Rv0"):
            pd0 = probs_to_buf(0)
            lo = [0, 0, 0, 4, 8, 12, 16, 16]
            region(2, 0, 2, 1, never, lambda n: pd0[lo[n]:lo[n + 1]])
        cp_wo(0).wait()
        def wo_cols(o, c0, c1, deps, first):
            wfn = lambda l, c: _nn(l, _b16(wo_p[:, (c0 + c) * 128:(c0 + c + 1) * 128]))
            return _mm_pinned(o, wfn, c1 - c0, deps, never, first=first)

        with jax.named_scope("Rv1"):
            v_half(0)
            rp = [_rowperm_into(wo_p, wo_raw, c) for c in range(4)]
            pd = probs_to_buf(HM)
            v_half(HM, lambda n: [pd[2 * n + 1]] + rp[n // 2][2 * (n % 2):2 * (n % 2) + 2])
            o0buf[...] = _w32(jnp.concatenate(_av(load_probs(0), vbuf, 0, None, None), axis=0))
            hbuf[0:HM, 0:KH] = _rows(xbuf, 0, HM)[:, 0:KH] + wo_cols(_b16(o0buf[...]), 0, 4, [], 1)
        cp_wo(1).wait()
        cp_x(1).wait()
        for c in range(4, 8):
            _rowperm_into(wo_p, wo_raw, c)
        o1 = _av(load_probs(HM), vbuf, HM, None, never)
        a0 = wo_cols(_b16(o0buf[...]), 4, 8, o1[:6], 1)
        hbuf[0:HM, KH:D] = _rows(xbuf, 0, HM)[:, KH:D] + a0
        xn_list = _ln_list(xbuf, TM, TM, lambda i: a0[0:8, 256:384], never)
        a1 = wo_cols(jnp.concatenate(o1, axis=0), 0, 8, xn_list[:14], 1)
        hbuf[HM:TM, :] = _rows(xbuf, HM, HM) + a1
        xn_scr[...] = _w32(jnp.concatenate(xn_list, axis=0))

    @jax.named_scope("A")
    def _attn(s, carry):
        @pl.when(s < NT - 1)
        def _():
            cp_x(s + 1).wait()
        never = zero_smem[0]
        for t in range(8):
            kbuf[t, 0:HALO, :] = kbuf[t, TM:TM + HALO, :]
            vbuf[t, 0:HALO, :] = vbuf[t, TM:TM + HALO, :]
        xn_list = _ln_list(xbuf, jnp.minimum(s + 1, NT - 1) * TM, TM)

        def kqv(r0, kdeps, qdeps):
            xn = _b16(xn_scr[r0 // 2:(r0 + HM) // 2, :])
            def proj(l, m, rows=slice(None)):
                return _nt(l[:, 0:KH], _b16(wta[m, rows, :])) + _nt(l[:, KH:D], _b16(wtb[m, rows, :]))
            k = _mm_pinned(xn, lambda l, c: proj(l, 1, slice(c * 64, (c + 1) * 64)), 8, kdeps, never)
            for t in range(8):
                kbuf[t, HALO + r0:HALO + r0 + HM, :] = k[:, t * 128:(t + 1) * 128]
            q = proj(_pin1(xn, qdeps, never), 0)
            v = proj(xn, 2)
            for t in range(8):
                vbuf[t, HALO + r0:HALO + r0 + HM, :] = v[:, t * 128:(t + 1) * 128]
            return lambda r: [q[r - r0:r - r0 + RB, j * 128:(j + 1) * 128] for j in range(8)]

        q0 = kqv(0, xn_list[:14], xn_list[14:])
        o0 = _av(_probs(q0, kbuf, 0, s * TM), vbuf, 0, never)
        q1 = kqv(HM, o0[:7], o0[7:])
        o1 = _av(_probs(q1, kbuf, HM, s * TM), vbuf, HM, never)
        xn_scr[...] = _w32(jnp.concatenate(xn_list, axis=0))
        nper = -(-(TM // LNB) // (NT - 1))
        blks = [jnp.minimum((s - 1) * nper + i, TM // LNB - 1) for i in range(nper)]
        hn_part = [_ln_list(hbuf, b * LNB, LNB)[0] for b in blks]
        wo_part(s, o0, o1, never, lambda a0: hn_part)
        for b, v in zip(blks, hn_part):
            hn_scr[pl.ds(pl.multiple_of(b * (LNB // 2), LNB // 2), LNB // 2), :] = _w32(v)
        return carry

    @jax.named_scope("B")
    def _ffn(t, carry):
        never = zero_smem[0]
        hn = _b16(hn_scr[...])
        hn_list = _ln_list(hbuf, jnp.minimum(t + 1, NT - 1) * TM, TM)
        acc = hbuf[tile_rows(t), :]
        off = 0
        for ci, fc in enumerate(BCH):
            cs = slice(off, off + fc)
            nq = fc // 128
            if ci == 0:
                g = _mm_pinned(hn, lambda l, n: _nn(l, _b16(wg[:, n * 128:(n + 1) * 128])), nq, hn_list[:6], never)
                u = _mm_pinned(hn, lambda l, n: _nn(l, _b16(wu[:, n * 128:(n + 1) * 128])), nq, hn_list[6:14], never, first=0)
            elif ci == 1:
                g = _nn(_pin1(hn, hn_list[14:], never), _b16(wg[:, cs]))
                u = _nn(hn, _b16(wu[:, cs]))
            else:
                g = _nn(hn, _b16(wg[:, cs]))
                u = _nn(hn, _b16(wu[:, cs]))
            a = _gelu_mul(g, u)
            if ci < len(BCH) - 1:
                acc = acc + _nn(a, _b16(wd[off // 2:(off + fc) // 2, :]))
            else:
                hn_scr[...] = _w32(jnp.concatenate(hn_list, axis=0))
                for h in range(len(OCUTS) - 1):
                    cs = slice(OCUTS[h], OCUTS[h + 1])
                    out = acc[:, cs] + _nn(a, _b16(wd[off // 2:(off + fc) // 2, cs]))
                    obuf[tile_rows(t), cs] = out.astype(bf16)
                    cp_o(t, h).start()
            off += fc
        return carry

    _first()
    lax.fori_loop(1, NT, _attn, 0)
    with jax.named_scope("trans"):
        for c in cp_ffn():
            c.wait()
    lax.fori_loop(0, NT, _ffn, 0)
    pltpu.make_async_copy(obuf, o_hbm, osem).wait()


@jax.jit
def pallas_sequential_preLN__sliding_local_dilated__glu_gated_geglu__prompt_kernel(
        A_x, A_wqkv, A_wo, B_x, B_w_gate, B_w_up, B_w_down):
    x = A_x.reshape(S, D)
    anyspec = pl.BlockSpec(memory_space=pl.ANY)
    out = pl.pallas_call(
        kernel,
        in_specs=[anyspec] * 6,
        out_specs=anyspec,
        out_shape=jax.ShapeDtypeStruct((S, D), bf16),
        scratch_shapes=[
            pltpu.VMEM((S, D), bf16),
            pltpu.VMEM((S // 2, D), u32),
            pltpu.VMEM((2, 3, KH // 2, D), u32),
            pltpu.VMEM((D // 2, D), u32),
            pltpu.VMEM((3, D // 2, KH), u32),
            pltpu.VMEM((3, D // 2, KH), u32),
            pltpu.VMEM((D // 2, D), u32),
            pltpu.VMEM((D // 2, DF), u32),
            pltpu.VMEM((D // 2, DF), u32),
            pltpu.VMEM((DF // 2, D), u32),
            pltpu.VMEM((TM // 2, D), u32),
            pltpu.VMEM((HM // 2, D), u32),
            pltpu.VMEM((W, TM, 128), f32),
            pltpu.VMEM((3, 8, TM + HALO, 128), f32),
            pltpu.VMEM((S, D), f32),
            pltpu.VMEM((TM // 2, D), u32),
            pltpu.SMEM((1,), jnp.int32),
            pltpu.SemaphoreType.DMA((11 + NT,)),
            pltpu.SemaphoreType.DMA,
        ],
        compiler_params=pltpu.CompilerParams(vmem_limit_bytes=110 * 1024 * 1024),
    )(x, A_wqkv, A_wo, B_w_gate, B_w_up, B_w_down)
    return out.reshape(1, S, D)
```

```python
import jax
import jax.numpy as jnp
from jax import lax
from jax.experimental import pallas as pl
from jax.experimental.pallas import tpu as pltpu

S, D, DF = 2048, 1024, 3584
DH, W, DIL = 32, 8, 2
TM = 256
HM = 128
NT = S // TM
RB = 8
LNB = 16
HALO = 16
KH = D // 2
SCALE = DH ** -0.5
LOG2E = 1.4426950408889634
MASK_RAW = -1e9 / SCALE
f32, bf16, u32 = jnp.float32, jnp.bfloat16, jnp.uint32

SKEW = (3, 3, 1, 1)
BCH = (1536, 1536, 512)
OCUTS = (0, 512, 896, 1024)


def _b16(x32):
    return pltpu.bitcast(x32, bf16)


def _w32(x16):
    return pltpu.bitcast(x16, u32)


def _nt(a, b):
    return lax.dot_general(a, b, (((1,), (1,)), ((), ())), preferred_element_type=f32)


def _nn(a, b):
    return jnp.dot(a, b, preferred_element_type=f32)


def _ln(x):
    m = jnp.mean(x, axis=-1, keepdims=True)
    xc = x - m
    v = jnp.mean(xc * xc, axis=-1, keepdims=True)
    return xc * lax.rsqrt(v + 1e-5)


def _rows(ref, row0, n):
    return ref[pl.ds(pl.multiple_of(row0, LNB), n), :].astype(f32)


def _ln_list(ref, row0, n, after=None, never=None):
    out = []
    for i, r in enumerate(range(0, n, LNB)):
        x = _rows(ref, row0 + r, LNB)
        if after is not None:
            nv = lax.broadcasted_iota(jnp.int32, (8, 128), 1) < never
            top = jnp.concatenate([jnp.where(nv, after(i), x[0:8, 0:128]), x[0:8, 128:]], axis=1)
            x = jnp.concatenate([top, x[8:]], axis=0)
        out.append(_ln(x).astype(bf16))
    return out


def _pin1(a, deps, never):
    if not deps:
        return a
    a32 = _w32(a)
    nv = lax.broadcasted_iota(jnp.int32, (8, 128), 1) < never
    top = []
    for t in range(a.shape[1] // 128):
        x = a32[0:8, t * 128:(t + 1) * 128]
        if t < len(deps):
            x = jnp.where(nv, _w32(deps[t])[0:8, t * 128:(t + 1) * 128], x)
        top.append(x)
    return _b16(jnp.concatenate([jnp.concatenate(top, axis=1), a32[8:]], axis=0))


def _mm_pinned(lhs, wfn, nchunks, deps, never, first=1):
    outs = []
    per = -(-len(deps) // (nchunks - first)) if deps else 0
    for c in range(nchunks):
        d = deps[(c - first) * per:(c - first + 1) * per] if (c >= first and deps) else []
        outs.append(wfn(_pin1(lhs, d, never), c))
    return jnp.concatenate(outs, axis=1)


def _perm_stage(blk, idx, stage):
    C = blk[idx[0]].shape[1]
    if stage < 3:
        s, ab = ((4, 2), (2, 4), (1, 8))[stage]
        bit = (lax.broadcasted_iota(jnp.int32, (8, C), 0) & s) != 0
        for a in idx:
            if a & ab:
                continue
            A, B = blk[a], blk[a | ab]
            blk[a] = jnp.where(bit, pltpu.roll(B, s, 0), A)
            blk[a | ab] = jnp.where(bit, B, pltpu.roll(A, 8 - s, 0))
    else:
        for a in idx:
            if a & 16:
                continue
            A, B = blk[a], blk[a | 16]
            blk[a] = (A & jnp.uint32(0xFFFF)) | (B << 16)
            blk[a | 16] = (A >> 16) | (B & jnp.uint32(0xFFFF0000))


def _perm_dest(a):
    return (a & 7) * 8 + ((a >> 3) & 1) * 4 + ((a >> 4) & 1) * 2 + (a >> 5)


def _perm_units(blk, half, store):
    C = blk[32 * half].shape[1]
    for a0 in range(2):
        idx = [a for a in range(32 * half, 32 * half + 32) if (a & 1) == a0]
        for t in range(C // 128):
            u = {a: blk[a][:, t * 128:(t + 1) * 128] for a in idx}
            for stage in range(4):
                _perm_stage(u, idx, stage)
            for a in idx:
                store(_perm_dest(a), t, u[a])


def _rowperm_into(dst, src, c):
    done = []
    for half in range(2):
        blk = {a: _w32(src[a * 16:(a + 1) * 16, c * 128:(c + 1) * 128]) for a in range(32 * half, 32 * half + 32)}

        def store(d, t, val):
            dst[d * 8:(d + 1) * 8, c * 128:(c + 1) * 128] = val
            done.append(val)
        _perm_units(blk, half, store)
    return done[15::16]


def _shifted(buf, j, r, w, zero):
    base = HALO + r - DIL * w
    if w >= 4 and zero is not None:
        return buf[j, pl.ds(base + zero, RB), :]
    return buf[j, base:base + RB, :]


def _probs_steps(q_rows, kbuf, r0, nrows, row0_global, sink, zero=None):
    nb = nrows // RB
    st = [dict() for _ in range(nb)]

    def s1(b):
        r = r0 + b * RB
        q = q_rows(r)
        ps = []
        for w in range(W):
            p = q[0] * _shifted(kbuf, 0, r, w, zero)
            for j in range(1, 8):
                p = p + q[j] * _shifted(kbuf, j, r, w, zero)
            ps.append(p)
        st[b]["p"] = ps
        st[b]["r"] = [pltpu.roll(p, 64, 1) for p in ps]

    def s2(b):
        ps = [p + r for p, r in zip(st[b]["p"], st[b]["r"])]
        st[b]["p"] = ps
        st[b]["r"] = [pltpu.roll(p, 32, 1) for p in ps]

    def s3(b):
        r = r0 + b * RB
        ls = [p + x for p, x in zip(st[b]["p"], st[b]["r"])]
        if r < HALO:
            row = row0_global + r + lax.broadcasted_iota(jnp.int32, (RB, 128), 0)
            ls = [ls[0]] + [jnp.where(row >= DIL * w, ls[w], MASK_RAW) for w in range(1, W)]
        m = ls[0]
        for w in range(1, W):
            m = jnp.maximum(m, ls[w])
        st[b]["e"] = [jnp.exp2((l - m) * (SCALE * LOG2E)) for l in ls]

    def s4(b):
        es = st[b]["e"]
        den = es[0]
        for w in range(1, W):
            den = den + es[w]
        st[b]["inv"] = 1.0 / den

    def s5(b):
        sink(b, [e * st[b]["inv"] for e in st[b]["e"]])

    stages = [s1, s2, s3, s4, s5]
    offs = [0]
    for sk in SKEW:
        offs.append(offs[-1] + sk)
    steps = []
    for t in range(nb + offs[-1]):
        def step(t=t):
            for si in reversed(range(5)):
                b = t - offs[si]
                if 0 <= b < nb:
                    stages[si](b)
        steps.append(step)
    return steps


def _probs(q_rows, kbuf, r0, row0_global, zero=None):
    out = [None] * (HM // RB)

    def sink(b, ps):
        out[b] = ps
    for f in _probs_steps(q_rows, kbuf, r0, HM, row0_global, sink, zero):
        f()
    return out


def _av_block(ps2, vbuf, r, never, zero=None):
    halves = []
    for e in range(2):
        rr = r + e * RB
        ps = ps2[e]
        if never is not None:
            nv = lax.broadcasted_iota(jnp.int32, (RB, 128), 1) < never
            last = vbuf[7, HALO + rr:HALO + rr + RB, :]
            ps = [jnp.where(nv, last, p) for p in ps]
        os_ = []
        for j in range(8):
            acc = None
            for w in range(W):
                t = ps[w] * _shifted(vbuf, j, rr, w, zero)
                acc = t if acc is None else acc + t
            os_.append(acc)
        halves.append(jnp.concatenate(os_, axis=1))
    return jnp.concatenate(halves, axis=0).astype(bf16)


def _av(ps, vbuf, r0, never, zero=None):
    return [_av_block(ps[i:i + 2], vbuf, r0 + i * RB, never, zero) for i in range(0, len(ps), 2)]


def _gelu_mul(g, u):
    c = 0.7978845608028654
    t = jnp.tanh(g * (c + (c * 0.044715) * (g * g)))
    return (0.5 * g * (1.0 + t) * u).astype(bf16)


def kernel(x_hbm, wqkv_hbm, wo_hbm, wg_hbm, wu_hbm, wd_hbm, o_hbm,
           obuf, xbuf, wraw, wo_raw, wta, wtb, wo_p, wg, wu, wd, xn_scr, qkv,
           hbuf, hn_scr, zero_smem, sems, osem):
    kbuf = qkv.at[1]
    vbuf = qkv.at[2]

    def tile_rows(t):
        return pl.ds(pl.multiple_of(t * TM, TM), TM)

    def cp_x(t):
        return pltpu.make_async_copy(x_hbm.at[tile_rows(t), :], xbuf.at[tile_rows(t), :], sems.at[11 + t])

    def cp_w(m, kh):
        cols = pl.ds(pl.multiple_of(m * D, D), D)
        return pltpu.make_async_copy(wqkv_hbm.at[kh * KH:(kh + 1) * KH, cols], wraw.at[kh, m], sems.at[2 * m + kh])

    def cp_wo(h):
        cs = slice(h * KH, (h + 1) * KH)
        return pltpu.make_async_copy(wo_hbm.at[:, cs], wo_raw.at[:, cs], sems.at[6 + h])

    def cp_ffn():
        return [pltpu.make_async_copy(wg_hbm, wg, sems.at[8]),
                pltpu.make_async_copy(wu_hbm, wu, sems.at[9]),
                pltpu.make_async_copy(wd_hbm, wd, sems.at[10])]

    def cp_o(t, h):
        cs = slice(OCUTS[h], OCUTS[h + 1])
        return pltpu.make_async_copy(obuf.at[tile_rows(t), cs], o_hbm.at[tile_rows(t), cs], osem)

    def wo_part(s, o0, o1, never, deps1=None):
        o0f = jnp.concatenate(o0, axis=0)
        o1f = jnp.concatenate(o1, axis=0)
        rows0 = pl.ds(pl.multiple_of(s * TM, HM), HM)
        rows1 = pl.ds(pl.multiple_of(s * TM + HM, HM), HM)
        wfn = lambda l, c: _nn(l, _b16(wo_p[:, c * 128:(c + 1) * 128]))
        a0 = _mm_pinned(o0f, wfn, 8, o1[:6], never, first=2)
        hbuf[rows0, :] = _rows(xbuf, s * TM, HM) + a0
        deps1 = deps1(a0) if deps1 is not None else []
        a1 = _mm_pinned(o1f, wfn, 8, deps1[:14], never)
        hbuf[rows1, :] = _rows(xbuf, s * TM + HM, HM) + a1
        return deps1

    def setup(m, kh, never, start=None):
        dst = (wta, wtb)[kh]
        blk = [None] * 64
        for c in range(8):
            raw = wraw[kh, m, :, c * 128:(c + 1) * 128]
            if start is not None:
                r32 = _w32(raw)
                nv = lax.broadcasted_iota(jnp.int32, (8, 128), 1) < never
                d = pltpu.bitcast(start(c), u32)
                parts = []
                for r in range(0, r32.shape[0], 64):
                    parts += [jnp.where(nv, d, r32[r:r + 8]), r32[r + 8:r + 64]]
                raw = _b16(jnp.concatenate(parts, axis=0))
            t32 = _w32(raw.T)
            for a in range(8):
                blk[c * 8 + a] = t32[a * 8:(a + 1) * 8, :]
        done = []

        def store(d, t, val):
            dst[m, d * 8:(d + 1) * 8, t * 128:(t + 1) * 128] = val
            done.append(val)
        for h in range(2):
            _perm_units(blk, h, store)
        return done[3::4]

    def region(m, kh, m_next, kh_next, never, extra=lambda n: []):
        wsrc = (wta, wtb)[kh]
        res = {}

        def tile(n, deps=()):
            lhs = xn_scr[:, kh * KH:(kh + 1) * KH]
            if deps:
                nv = lax.broadcasted_iota(jnp.int32, (8, 128), 1) < never
                rows = []
                for rr in range(lhs.shape[0] // 8):
                    tiles = []
                    for t in range(lhs.shape[1] // 128):
                        x = lhs[rr * 8:(rr + 1) * 8, t * 128:(t + 1) * 128]
                        k = rr * (lhs.shape[1] // 128) + t
                        if k < len(deps):
                            x = jnp.where(nv, deps[k][:, 0:128], x)
                        tiles.append(x)
                    rows.append(jnp.concatenate(tiles, axis=1))
                lhs = jnp.concatenate(rows, axis=0)
            r = _nt(_b16(lhs), _b16(wsrc[m, n * 64:(n + 1) * 64, :]))
            res[n] = r[0:8]
            if kh == 1:
                r = r + qkv[m, n, HALO:HALO + TM, :]
            qkv[m, n, HALO:HALO + TM, :] = r

        for n in range(7):
            tile(n, extra(n))
        blk = setup(m_next, kh_next, never, lambda c: res[c // 4])
        tile(7, blk)

    @jax.named_scope("P")
    def _first():
        zero_smem[0] = 0
        never = zero_smem[0]
        cp_x(0).start()
        cp_w(0, 0).start()
        cp_x(0).wait()
        for c in ([cp_w(0, 1)] + [cp_w(m, kh) for m in (1, 2) for kh in (0, 1)] + [cp_wo(0), cp_wo(1)]
                  + [cp_x(t) for t in range(1, NT)] + cp_ffn()):
            c.start()
        def ln0(i, carry):
            r = i * 64
            xn_scr[pl.ds(pl.multiple_of(i * 32, 32), 32), :] = _w32(jnp.concatenate(_ln_list(xbuf, r, 64), axis=0))
            return carry
        lax.fori_loop(0, TM // 64, ln0, 0)
        for t in range(8):
            kbuf[t, 0:HALO, :] = jnp.zeros((HALO, 128), f32)
            vbuf[t, 0:HALO, :] = jnp.zeros((HALO, 128), f32)
        cp_w(0, 0).wait()

        def setup0(i, carry):
            h = lax.shift_right_logical(i, 1)
            k0 = pl.multiple_of((i & 1) * (KH // 2), KH // 2)
            blk = {}
            for c in range(4):
                raw = wraw[0, 0, pl.ds(k0, KH // 2), pl.ds(pl.multiple_of((4 * h + c) * 128, 128), 128)]
                t32 = _w32(raw.T)
                for a in range(8):
                    blk[c * 8 + a] = t32[a * 8:(a + 1) * 8, :]

            def store(d, t, val):
                wta[0, pl.ds(pl.multiple_of((d + h) * 8, 8), 8), pl.ds(pl.multiple_of(k0 + t * 128, 128), 128)] = val
            _perm_units(blk, 0, store)
            return carry
        lax.fori_loop(0, 4, setup0, 0)

        def body(m, carry):
            never = zero_smem[0]
            cp_w(m, 1).wait()
            region(m, 0, m, 1, never)

            @pl.when(m < 2)
            def _():
                cp_w(m + 1, 0).wait()
            region(m, 1, jnp.minimum(m + 1, 2), 0, never)
            return carry
        with jax.named_scope("Ploop"):
            lax.fori_loop(0, 3, body, 0)

        cp_wo(0).wait()
        cp_wo(1).wait()
        cp_x(1).wait()
        never = zero_smem[0]

        def q_rows(r):
            return [qkv[0, t, HALO + r:HALO + r + RB, :] for t in range(8)]
        o0 = _av(_probs(q_rows, kbuf, 0, 0, never), vbuf, 0, None, never)
        for c in range(8):
            _rowperm_into(wo_p, wo_raw, c)
        o1 = _av(_probs(q_rows, kbuf, HM, 0, never), vbuf, HM, None, never)
        xn_list = wo_part(0, o0, o1, never, lambda a0: _ln_list(xbuf, TM, TM, lambda i: a0[0:8, 896:1024], never))
        xn_scr[...] = _w32(jnp.concatenate(xn_list, axis=0))

    @jax.named_scope("A")
    def _attn(s, carry):
        @pl.when(s < NT - 1)
        def _():
            cp_x(s + 1).wait()
        never = zero_smem[0]
        for t in range(8):
            kbuf[t, 0:HALO, :] = kbuf[t, TM:TM + HALO, :]
            vbuf[t, 0:HALO, :] = vbuf[t, TM:TM + HALO, :]
        xn_list = _ln_list(xbuf, jnp.minimum(s + 1, NT - 1) * TM, TM)

        def kqv(r0, kdeps, qdeps):
            xn = _b16(xn_scr[r0 // 2:(r0 + HM) // 2, :])
            def proj(l, m, rows=slice(None)):
                return _nt(l[:, 0:KH], _b16(wta[m, rows, :])) + _nt(l[:, KH:D], _b16(wtb[m, rows, :]))
            k = _mm_pinned(xn, lambda l, c: proj(l, 1, slice(c * 64, (c + 1) * 64)), 8, kdeps, never)
            for t in range(8):
                kbuf[t, HALO + r0:HALO + r0 + HM, :] = k[:, t * 128:(t + 1) * 128]
            q = proj(_pin1(xn, qdeps, never), 0)
            v = proj(xn, 2)
            for t in range(8):
                vbuf[t, HALO + r0:HALO + r0 + HM, :] = v[:, t * 128:(t + 1) * 128]
            return lambda r: [q[r - r0:r - r0 + RB, j * 128:(j + 1) * 128] for j in range(8)]

        q0 = kqv(0, xn_list[:14], xn_list[14:])
        o0 = _av(_probs(q0, kbuf, 0, s * TM), vbuf, 0, never)
        q1 = kqv(HM, o0[:7], o0[7:])
        o1 = _av(_probs(q1, kbuf, HM, s * TM), vbuf, HM, never)
        xn_scr[...] = _w32(jnp.concatenate(xn_list, axis=0))
        nper = -(-(TM // LNB) // (NT - 1))
        blks = [jnp.minimum((s - 1) * nper + i, TM // LNB - 1) for i in range(nper)]
        hn_part = [_ln_list(hbuf, b * LNB, LNB)[0] for b in blks]
        wo_part(s, o0, o1, never, lambda a0: hn_part)
        for b, v in zip(blks, hn_part):
            hn_scr[pl.ds(pl.multiple_of(b * (LNB // 2), LNB // 2), LNB // 2), :] = _w32(v)
        return carry

    @jax.named_scope("B")
    def _ffn(t, carry):
        never = zero_smem[0]
        hn = _b16(hn_scr[...])
        hn_list = _ln_list(hbuf, jnp.minimum(t + 1, NT - 1) * TM, TM)
        acc = hbuf[tile_rows(t), :]
        off = 0
        for ci, fc in enumerate(BCH):
            cs = slice(off, off + fc)
            nq = fc // 128
            if ci == 0:
                g = _mm_pinned(hn, lambda l, n: _nn(l, wg[:, n * 128:(n + 1) * 128]), nq, hn_list[:6], never)
                u = _mm_pinned(hn, lambda l, n: _nn(l, wu[:, n * 128:(n + 1) * 128]), nq, hn_list[6:14], never, first=0)
            elif ci == 1:
                g = _nn(_pin1(hn, hn_list[14:], never), wg[:, cs])
                u = _nn(hn, wu[:, cs])
            else:
                g = _nn(hn, wg[:, cs])
                u = _nn(hn, wu[:, cs])
            a = _gelu_mul(g, u)
            if ci < len(BCH) - 1:
                acc = acc + _nn(a, wd[cs, :])
            else:
                hn_scr[...] = _w32(jnp.concatenate(hn_list, axis=0))
                for h in range(len(OCUTS) - 1):
                    oc = slice(OCUTS[h], OCUTS[h + 1])
                    out = acc[:, oc] + _nn(a, wd[cs, oc])
                    obuf[tile_rows(t), oc] = out.astype(bf16)
                    cp_o(t, h).start()
            off += fc
        return carry

    _first()
    lax.fori_loop(1, NT, _attn, 0)
    with jax.named_scope("trans"):
        for c in cp_ffn():
            c.wait()
    lax.fori_loop(0, NT, _ffn, 0)
    pltpu.make_async_copy(obuf, o_hbm, osem).wait()


@jax.jit
def pallas_sequential_preLN__sliding_local_dilated__glu_gated_geglu__prompt_kernel(
        A_x, A_wqkv, A_wo, B_x, B_w_gate, B_w_up, B_w_down):
    x = A_x.reshape(S, D)
    anyspec = pl.BlockSpec(memory_space=pl.ANY)
    out = pl.pallas_call(
        kernel,
        in_specs=[anyspec] * 6,
        out_specs=anyspec,
        out_shape=jax.ShapeDtypeStruct((S, D), bf16),
        scratch_shapes=[
            pltpu.VMEM((S, D), bf16),
            pltpu.VMEM((S, D), bf16),
            pltpu.VMEM((2, 3, KH, D), bf16),
            pltpu.VMEM((D, D), bf16),
            pltpu.VMEM((3, D // 2, KH), u32),
            pltpu.VMEM((3, D // 2, KH), u32),
            pltpu.VMEM((D // 2, D), u32),
            pltpu.VMEM((D, DF), bf16),
            pltpu.VMEM((D, DF), bf16),
            pltpu.VMEM((DF, D), bf16),
            pltpu.VMEM((TM // 2, D), u32),
            pltpu.VMEM((3, 8, TM + HALO, 128), f32),
            pltpu.VMEM((S, D), f32),
            pltpu.VMEM((TM // 2, D), u32),
            pltpu.SMEM((1,), jnp.int32),
            pltpu.SemaphoreType.DMA((11 + NT,)),
            pltpu.SemaphoreType.DMA,
        ],
        compiler_params=pltpu.CompilerParams(vmem_limit_bytes=110 * 1024 * 1024),
    )(x, A_wqkv, A_wo, B_w_gate, B_w_up, B_w_down)
    return out.reshape(1, S, D)
```
